```python
import os as _os
_os.environ.setdefault("JAX_PLATFORMS", "cpu")
import jax
import jax.numpy as jnp

def _softmax(x, axis=-1):
    return jax.nn.softmax(x, axis=axis)
def _gelu(x):
    return jax.nn.gelu(x, approximate=True)
def _silu(x):
    return jax.nn.silu(x)
def _sigmoid(x):
    return jax.nn.sigmoid(x)
def _layernorm(x, axis=-1, eps=1e-5):
    m = jnp.mean(x, axis=axis, keepdims=True)
    v = jnp.var(x, axis=axis, keepdims=True)
    return (x - m) / jnp.sqrt(v + eps)
def _scatter_add(tgt, idx, src, axis=0):
    return tgt.at[idx].add(src)
def _segment_sum(src, seg, n):
    return jax.ops.segment_sum(src, seg, n)
class _Rng:
    def __init__(self, key):
        self._k = key
    def _next(self):
        self._k, sub = jax.random.split(self._k)
        return sub
    def normal(self, shape):
        return jax.random.normal(self._next(), shape, dtype=jnp.bfloat16)
    def randint(self, lo, hi, shape):
        return jax.random.randint(self._next(), shape, lo, hi, dtype=jnp.int32)
    def uniform(self, shape, lo=0.0, hi=1.0):
        return jax.random.uniform(self._next(), shape, jnp.bfloat16, lo, hi)
    def permutation(self, n):
        return jax.random.permutation(self._next(), n)


kernel_name = 'interleave_layers__softmax_full_mha__glu_gated_bilinear__prompt'

def setup_inputs():
    _rng = _Rng(jax.random.key(int.from_bytes(__import__("os").urandom(4), "little")))
    _w = (lambda a: (lambda t: t.astype(jnp.bfloat16) if jnp.issubdtype(t.dtype, jnp.floating) else t)(jnp.asarray(a)))
    def _A_setup():
        B, S, D = 1, 2048, 512
        return {
            "x": _w((lambda *s: _rng.normal(s) * 0.05)(B, S, D)),
            "wqkv": _w((lambda *s: _rng.normal(s) * 0.05)(D, 3 * D)),
            "wo": _w((lambda *s: _rng.normal(s) * 0.05)(D, D)),
        }
    _A_in = _A_setup()

    def _B_setup():
        B, S, D, F = 1, 2048, 512, 1792
        return {
            "x": _w((lambda *s: _rng.normal(s) * 0.05)(B, S, D)),
            "w_gate": _w((lambda *s: _rng.normal(s) * 0.4)(D, F) * (D ** -0.5)),
            "w_up": _w((lambda *s: _rng.normal(s) * 0.4)(D, F) * (D ** -0.5)),
            "w_down": _w((lambda *s: _rng.normal(s) * 0.4)(F, D) * (F ** -0.5)),
        }
    _B_in = _B_setup()

    return {
        "A_x": _A_in["x"],
        "A_wqkv": _A_in["wqkv"],
        "A_wo": _A_in["wo"],
        "B_x": _B_in["x"],
        "B_w_gate": _B_in["w_gate"],
        "B_w_up": _B_in["w_up"],
        "B_w_down": _B_in["w_down"],
    }

def reference(A_x, A_wqkv, A_wo, B_x, B_w_gate, B_w_up, B_w_down):
    def _A_ref(x, wqkv, wo):
        B, S, D = x.shape
        H = 32; Dh = D // H
        qkv = (lambda x, *d: x.transpose(*d))((x @ wqkv).reshape(B, S, 3, H, Dh), 2, 0, 3, 1, 4)
        q, k, v = qkv[0], qkv[1], qkv[2]
        scale = Dh ** -0.5
        scores = jnp.einsum("bhqd,bhkd->bhqk", q, k) * scale
        p = _softmax(scores, axis=-1)
        o = jnp.einsum("bhqk,bhkd->bhqd", p, v)
        return (lambda x, *d: x.transpose(*d))(o, 0, 2, 1, 3).reshape(B, S, D) @ wo

    def _B_ref(x, w_gate, w_up, w_down):
        g = jnp.einsum("bsd,df->bsf", x, w_gate)
        u = jnp.einsum("bsd,df->bsf", x, w_up)
        h = g * u
        return jnp.einsum("bsf,fd->bsd", h, w_down)

    x = A_x
    x = x + _A_ref(_layernorm(x, axis=-1), A_wqkv, A_wo)
    x = x + _B_ref(_layernorm(x, axis=-1), B_w_gate, B_w_up, B_w_down)
    x = x + _A_ref(_layernorm(x, axis=-1), A_wqkv, A_wo)
    x = x + _B_ref(_layernorm(x, axis=-1), B_w_gate, B_w_up, B_w_down)
    return x
```

```python
import functools
import math

import jax
import jax.numpy as jnp
from jax import lax
import jax.experimental.pallas as pl
import jax.experimental.pallas.tpu as pltpu

F32 = jnp.float32
BF16 = jnp.bfloat16

N_HEADS = 32
N_LAYERS = 2
LN_EPS = 1e-5

QB = 512
CK = 128
SUB = 4
LAG = 6
SKEW = 2
RB = 512
FB = 256


def _layernorm(x):
    m = jnp.mean(x, axis=-1, keepdims=True)
    xc = x - m
    v = jnp.mean(xc * xc, axis=-1, keepdims=True)
    return xc * lax.rsqrt(v + LN_EPS)


def _kernel(x_in, wqkv, wo, wg, wu, wd, out_ref,
            x_ref, k_ref, qt_ref, vt_ref, o_ref, h_ref,
            s00, s01, s10, s11, m_ref, z_ref, *, S, D, F):
    dh = D // N_HEADS
    gph = 128 // dh
    nqb = S // QB
    nc = S // CK
    half = nc // 2
    sr = CK // SUB
    nit = (N_HEADS // gph) * nqb
    qscale = (dh ** -0.5) * math.log2(math.e)
    sb = ((s00, s01), (s10, s11))

    z_ref[0] = 0
    z_ref[1] = 0

    def qkv_block(i, x):
        rows = pl.ds(pl.multiple_of(i * RB, RB), RB)
        ln = _layernorm(x).astype(BF16)
        q = jnp.dot(ln, wqkv[:, 0:D], preferred_element_type=F32) * qscale
        qt_ref[:, rows] = q.T.astype(BF16)
        k = jnp.dot(ln, wqkv[:, D:2 * D], preferred_element_type=F32)
        k_ref[rows, :] = k.astype(BF16)
        v = jnp.dot(ln, wqkv[:, 2 * D:3 * D], preferred_element_type=F32)
        vt_ref[:, rows] = v.T.astype(BF16)

    def ffn_block(i):
        rows = pl.ds(pl.multiple_of(i * RB, RB), RB)
        x = x_ref[rows, :] + jnp.dot(o_ref[rows, :], wo[...], preferred_element_type=F32)
        ln = _layernorm(x).astype(BF16)
        for n in range(0, F, FB):
            g = jnp.dot(ln, wg[:, n:n + FB], preferred_element_type=F32)
            u = jnp.dot(ln, wu[:, n:n + FB], preferred_element_type=F32)
            h_ref[:, n:n + FB] = (g * u).astype(BF16)
        return x + jnp.dot(h_ref[...], wd[...], preferred_element_type=F32)

    def wq(it, g):
        t = it // nqb
        qb = it % nqb
        row = pl.multiple_of(t * 128 + g * dh, dh)
        col = pl.multiple_of(qb * QB, QB)
        q = qt_ref[pl.ds(row, dh), pl.ds(col, QB)]
        parts = []
        if g > 0:
            parts.append(jnp.zeros((g * dh, QB), BF16))
        parts.append(q)
        if g < gph - 1:
            parts.append(jnp.zeros(((gph - 1 - g) * dh, QB), BF16))
        return jnp.concatenate(parts, axis=0)

    def qk_chunk(w, it, par, c, m, z, hist):
        t = it // nqb
        kc = k_ref[c * CK:(c + 1) * CK, pl.ds(pl.multiple_of(t * 128, 128), 128)]
        s = jnp.dot(kc, w, preferred_element_type=F32)
        sb[par][c // half][pl.ds(pl.multiple_of(z + (c % half) * CK, 8), CK), :] = s
        for r in range(CK // 8):
            s8 = s[r * 8:(r + 1) * 8]
            m = s8 if m is None else jnp.maximum(m, s8)
            if (r + 1) % (sr // 8) == 0:
                hist.append(m)
        return m

    def pv_chunk(it, g, c, mb, l, o, z0, z1, j, hist):
        t = it // nqb
        ref = sb[g % 2][c // half]
        ps = [None] * (CK // 16)
        for si in range(SUB):
            sub = SUB - 1 - si
            js = j * SUB + si
            mbc = mb
            if js >= LAG:
                mbc = jnp.where(z0 == 0, mb, hist[js - LAG])
            for rr in reversed(range(sr // 16)):
                r16 = sub * (sr // 16) + rr
                s = ref[pl.ds(pl.multiple_of(z1 + (c % half) * CK + r16 * 16, 8), 16), :]
                p = jnp.exp2(s.reshape(2, 8, QB) - mbc[None])
                p2 = p[0] + p[1]
                l = p2 if l is None else l + p2
                ps[r16] = p.reshape(16, QB)
        pb = jnp.concatenate(ps, axis=0).astype(BF16)
        row = pl.multiple_of(t * 128 + g * dh, dh)
        v = vt_ref[pl.ds(row, dh), c * CK:(c + 1) * CK]
        oc = jnp.dot(v, pb, preferred_element_type=F32)
        o = oc if o is None else o + oc
        return l, o

    def finish_max(m):
        return jnp.broadcast_to(jnp.max(m, axis=0, keepdims=True), (8, QB))

    def attention():
        w = wq(0, 0)
        m = None
        for c in range(nc):
            m = qk_chunk(w, 0, 0, c, m, 0, [])
        m_ref[0] = finish_max(m)
        w = wq(0, 1)
        m = None
        for c in range(SKEW):
            m = qk_chunk(w, 0, 1, c, m, 0, [])
        m_ref[1] = m

        def body(it, carry):
            z0 = z_ref[0]
            z1 = z_ref[1]
            nxt = jnp.minimum(it + 1, nit - 1)
            mfin = {0: m_ref[0]}
            m = m_ref[1]
            w = None
            hist = []
            l = o = None
            outs = []
            for j in range(gph * nc):
                jq = j + nc + SKEW
                gq, cq = jq // nc, jq % nc
                itq = it if gq < gph else nxt
                if cq == 0:
                    m = None
                if cq == 0 or w is None:
                    w = wq(itq, gq % gph)
                m = qk_chunk(w, itq, gq % 2, cq, m, z0, hist)
                if cq == nc - 1:
                    mfin[gq] = finish_max(m)
                g, c = j // nc, j % nc
                if c == 0:
                    l = o = None
                l, o = pv_chunk(it, g, c, mfin[g], l, o, z0, z1, j, hist)
                if c == nc - 1:
                    lt = jnp.sum(l, axis=0, keepdims=True)
                    outs.append(o / lt)
            m_ref[0] = mfin[gph]
            m_ref[1] = m
            t = it // nqb
            qb = it % nqb
            ot = jnp.concatenate(outs, axis=0)
            o_ref[pl.ds(pl.multiple_of(qb * QB, QB), QB),
                  pl.ds(pl.multiple_of(t * 128, 128), 128)] = ot.T.astype(BF16)
            return carry

        lax.fori_loop(0, nit, body, 0)

    def init_body(i, c):
        rows = pl.ds(pl.multiple_of(i * RB, RB), RB)
        x_ref[rows, :] = x_in[rows, :].astype(F32)
        return c

    lax.fori_loop(0, S // RB, init_body, 0)

    def layer(li, carry):
        def a_body(i, c):
            rows = pl.ds(pl.multiple_of(i * RB, RB), RB)
            qkv_block(i, x_ref[rows, :])
            return c

        lax.fori_loop(0, S // RB, a_body, 0)
        attention()

        def b_body(i, c):
            rows = pl.ds(pl.multiple_of(i * RB, RB), RB)
            y = ffn_block(i)
            x_ref[rows, :] = y
            out_ref[rows, :] = y.astype(out_ref.dtype)
            return c

        lax.fori_loop(0, S // RB, b_body, 0)
        return carry

    lax.fori_loop(0, N_LAYERS, layer, 0)


@jax.jit
def pallas_interleave_layers__softmax_full_mha__glu_gated_bilinear__prompt_kernel(
    A_x: jax.Array,
    A_wqkv: jax.Array,
    A_wo: jax.Array,
    B_x: jax.Array,
    B_w_gate: jax.Array,
    B_w_up: jax.Array,
    B_w_down: jax.Array,
):
    del B_x
    B, S, D = A_x.shape
    assert B == 1
    F = B_w_gate.shape[1]
    x2 = A_x.reshape(S, D)

    scratch = [
        pltpu.VMEM((S, D), F32),
        pltpu.VMEM((S, D), BF16),
        pltpu.VMEM((D, S), BF16),
        pltpu.VMEM((D, S), BF16),
        pltpu.VMEM((S, D), BF16),
        pltpu.VMEM((RB, F), BF16),
        pltpu.VMEM((S // 2, QB), F32),
        pltpu.VMEM((S // 2, QB), F32),
        pltpu.VMEM((S // 2, QB), F32),
        pltpu.VMEM((S // 2, QB), F32),
        pltpu.VMEM((2, 8, QB), F32),
        pltpu.SMEM((2,), jnp.int32),
    ]
    out = pl.pallas_call(
        functools.partial(_kernel, S=S, D=D, F=F),
        out_shape=jax.ShapeDtypeStruct((S, D), A_x.dtype),
        scratch_shapes=scratch,
        compiler_params=pltpu.CompilerParams(vmem_limit_bytes=100 * 1024 * 1024),
    )(x2, A_wqkv, A_wo, B_w_gate, B_w_up, B_w_down)
    return out.reshape(B, S, D)
```

```python
import functools
import math

import jax
import jax.numpy as jnp
from jax import lax
import jax.experimental.pallas as pl
import jax.experimental.pallas.tpu as pltpu

F32 = jnp.float32
BF16 = jnp.bfloat16

N_HEADS = 32
N_LAYERS = 2
LN_EPS = 1e-5

QB = 512
CK = 128
SUB = 4
LAG = 6
SKEW = 2
RB = 512
RS = 128
EPI = 2
LN2FFN = 1
FB = 256


def _layernorm(x):
    m = jnp.mean(x, axis=-1, keepdims=True)
    xc = x - m
    v = jnp.mean(xc * xc, axis=-1, keepdims=True)
    return xc * lax.rsqrt(v + LN_EPS)


def _kernel(x_hbm, wqkv_hbm, wo_hbm, wg_hbm, wu_hbm, wd_hbm, out_hbm,
            xio, wqkv, wo, wg, wu, wd,
            x_ref, ln_ref, k_ref, qt_ref, vt_ref, ot_ref, h_ref,
            s00, s01, s10, s11, m_ref, l_ref, oc_ref, z_ref, sems, *, S, D, F):
    dh = D // N_HEADS
    gph = 128 // dh
    nt = N_HEADS // gph
    nqb = S // QB
    nc = S // CK
    half = nc // 2
    sr = CK // SUB
    nit = nt * nqb
    nrb = S // RB
    lagc = nc + SKEW
    qscale = (dh ** -0.5) * math.log2(math.e)
    sb = ((s00, s01), (s10, s11))

    def x_copy(i):
        rows = pl.ds(pl.multiple_of(i * RB, RB), RB)
        return pltpu.make_async_copy(x_hbm.at[rows, :], xio.at[rows, :], sems.at[i])

    def out_copy(i):
        rows = pl.ds(pl.multiple_of(i * RB, RB), RB)
        return pltpu.make_async_copy(xio.at[rows, :], out_hbm.at[rows, :], sems.at[i])

    w_pairs = ((wqkv_hbm, wqkv), (wo_hbm, wo), (wg_hbm, wg), (wu_hbm, wu), (wd_hbm, wd))

    def w_copy(j):
        return pltpu.make_async_copy(w_pairs[j][0], w_pairs[j][1], sems.at[nrb + j])

    x_copy(0).start()
    w_copy(0).start()
    x_copy(1).start()

    z_ref[0] = 0
    z_ref[1] = 0
    s01[...] = jnp.zeros_like(s01)
    s10[...] = jnp.zeros_like(s10)
    s11[...] = jnp.zeros_like(s11)
    m_ref[...] = jnp.zeros_like(m_ref)
    l_ref[...] = jnp.zeros_like(l_ref)
    oc_ref[...] = jnp.zeros_like(oc_ref)
    x_ref[RB:, :] = jnp.zeros((S - RB, D), F32)
    x_copy(0).wait()
    x0 = xio[0:RB, :].astype(F32)
    x_ref[0:RB, :] = x0
    ln_ref[S:S + RB, :] = _layernorm(x0).astype(BF16)

    def blk(i):
        return pl.ds(pl.multiple_of(i * RB, RB), RB)

    def qkv_block(li, i):
        rows = blk(i)
        ln = ln_ref[blk(nrb + i), :]
        q = jnp.dot(ln, wqkv[:, 0:D], preferred_element_type=F32) * qscale
        qt_ref[:, rows] = q.T.astype(BF16)
        nxt = jnp.minimum(i + 1, nrb - 1)
        nrows = blk(nxt)
        x = jnp.where(li == 0, xio[nrows, :].astype(F32), x_ref[nrows, :])
        x_ref[nrows, :] = x
        ln_ref[blk(nrb + nxt), :] = _layernorm(x).astype(BF16)
        v = jnp.dot(ln, wqkv[:, 2 * D:3 * D], preferred_element_type=F32)
        vt_ref[:, rows] = v.T.astype(BF16)
        k = jnp.dot(ln, wqkv[:, D:2 * D], preferred_element_type=F32)
        k_ref[rows, :] = k.astype(BF16)

    def wo_pieces():
        for r in range(S // RS):
            rows = slice(r * RS, (r + 1) * RS)
            o = ot_ref[:, rows].T.astype(BF16)
            ys = []
            for n in range(0, D, 128):
                ys.append(jnp.dot(o, wo[:, n:n + 128], preferred_element_type=F32))
                if n + 128 == D:
                    x = x_ref[rows, :] + jnp.concatenate(ys, axis=1)
                    x_ref[rows, :] = x
                    if r < RB // RS or not LN2FFN:
                        ln_ref[rows, :] = _layernorm(x).astype(BF16)
                yield

    def ffn_block(i):
        rows = blk(i)
        z0 = z_ref[0]
        nxt = jnp.minimum(i + 1, nrb - 1)
        todo = [(nxt * RB + r * RS, 0) for r in range(RB // RS)] if LN2FFN else []
        todo += [((i % 2) * (RB // 2) + r * RS, S) for r in range(RB // 2 // RS)]
        ln0 = ln_ref[rows, :]
        for n in range(0, F, FB):
            ln = ln0
            if n > 0 and todo:
                src, off = todo.pop(0)
                xs = x_ref[pl.ds(pl.multiple_of(src, RS), RS), :]
                piece = _layernorm(xs).astype(BF16)
                ln_ref[pl.ds(pl.multiple_of(src + off, RS), RS), :] = piece
                ln = jnp.concatenate([jnp.where(z0 == 0, ln0[0:RS], piece), ln0[RS:]], axis=0)
            g = jnp.dot(ln, wg[:, n:n + FB], preferred_element_type=F32)
            u = jnp.dot(ln, wu[:, n:n + FB], preferred_element_type=F32)
            h_ref[:, n:n + FB] = (g * u).astype(BF16)
        assert not todo
        y = x_ref[rows, :] + jnp.dot(h_ref[...], wd[...], preferred_element_type=F32)
        x_ref[rows, :] = y
        xio[rows, :] = y.astype(xio.dtype)

    def head_row(it, g):
        return pl.multiple_of((it % nt) * 128 + g * dh, dh)

    def q_col(it):
        return pl.multiple_of((it // nt) * QB, QB)

    def wq(it, g):
        q = qt_ref[pl.ds(head_row(it, g), dh), pl.ds(q_col(it), QB)]
        parts = []
        if g > 0:
            parts.append(jnp.zeros((g * dh, QB), BF16))
        parts.append(q)
        if g < gph - 1:
            parts.append(jnp.zeros(((gph - 1 - g) * dh, QB), BF16))
        return jnp.concatenate(parts, axis=0)

    def qk_chunk(w, it, par, c, m, z, hist):
        kc = k_ref[c * CK:(c + 1) * CK, pl.ds(pl.multiple_of((it % nt) * 128, 128), 128)]
        s = jnp.dot(kc, w, preferred_element_type=F32)
        sb[par][c // half][pl.ds(pl.multiple_of(z + (c % half) * CK, 8), CK), :] = s
        for r in range(CK // 8):
            s8 = s[r * 8:(r + 1) * 8]
            m = s8 if m is None else jnp.maximum(m, s8)
            if (r + 1) % (sr // 8) == 0:
                hist.append(m)
        return m

    def pv_chunk(it, g, c, mb, l, o, z0, z1, j, hist):
        ref = sb[g % 2][c // half]
        ps = [None] * (CK // 16)
        for si in range(SUB):
            sub = SUB - 1 - si
            js = j * SUB + si
            mbc = mb
            if hist is not None and js >= LAG:
                mbc = jnp.where(z0 == 0, mb, hist[js - LAG])
            for rr in reversed(range(sr // 16)):
                r16 = sub * (sr // 16) + rr
                s = ref[pl.ds(pl.multiple_of(z1 + (c % half) * CK + r16 * 16, 8), 16), :]
                p = jnp.exp2(s.reshape(2, 8, QB) - mbc[None])
                p2 = p[0] + p[1]
                l = p2 if l is None else l + p2
                ps[r16] = p.reshape(16, QB)
        pb = jnp.concatenate(ps, axis=0).astype(BF16)
        v = vt_ref[pl.ds(head_row(it, g), dh), c * CK:(c + 1) * CK]
        oc = jnp.dot(v, pb, preferred_element_type=F32)
        o = oc if o is None else o + oc
        return l, o

    def pv_finish(it, g, l, o):
        lt = jnp.sum(l, axis=0, keepdims=True)
        ot_ref[pl.ds(head_row(it, g), dh), pl.ds(q_col(it), QB)] = o / lt

    def finish_max(m):
        return jnp.broadcast_to(jnp.max(m, axis=0, keepdims=True), (8, QB))

    def att_body(it, carry):
        z0 = z_ref[0]
        z1 = z_ref[1]
        prv = jnp.maximum(it - 1, 0)
        mfin = {-2: m_ref[0], -1: finish_max(m_ref[1])}
        l = l_ref[...]
        o = oc_ref[...]
        hist = []
        m = w = None
        for j in range(gph * nc):
            gq, cq = j // nc, j % nc
            if cq == 0:
                m = None
                w = wq(it, gq)
            m = qk_chunk(w, it, gq % 2, cq, m, z0, hist)
            if cq == nc - 1 and gq < gph - 1:
                mfin[gq] = finish_max(m)
            g, c = (j - lagc) // nc, (j - lagc) % nc
            itp = it if g >= 0 else prv
            if c == 0:
                l = o = None
            l, o = pv_chunk(itp, g % gph, c, mfin[g], l, o, z0, z1, j, hist)
            if c == nc - 1:
                pv_finish(itp, g % gph, l, o)
        m_ref[0] = mfin[gph - 2]
        m_ref[1] = m
        l_ref[...] = l
        oc_ref[...] = o
        return carry

    def att_epilogue():
        it = nit - 1
        l = l_ref[...]
        o = oc_ref[...]
        mfin = {gph - 2: m_ref[0], gph - 1: finish_max(m_ref[1])}
        pieces = wo_pieces()
        assert lagc * EPI <= (S - QB) // RS * (D // 128)
        for j in range(lagc):
            for _ in range(EPI):
                next(pieces)
            g, c = gph + (j - lagc) // nc, (j - lagc) % nc
            if c == 0:
                l = o = None
            l, o = pv_chunk(it, g, c, mfin[g], l, o, 0, 0, j, None)
            if c == nc - 1:
                pv_finish(it, g, l, o)
        for _ in pieces:
            pass

    def layer(li, carry):
        def a_body(i, c):
            @pl.when(li == 0)
            def _():
                @pl.when(i + 1 < nrb)
                def _():
                    x_copy(i + 1).wait()

                @pl.when(i == 0)
                def _():
                    w_copy(0).wait()
                    for b in range(2, nrb):
                        x_copy(b).start()

                @pl.when(i == 1)
                def _():
                    for j in range(1, 5):
                        w_copy(j).start()

            qkv_block(li, i)
            return c

        lax.fori_loop(0, nrb, a_body, 0)
        lax.fori_loop(0, nit, att_body, 0)

        @pl.when(li == 0)
        def _():
            for j in range(1, 5):
                w_copy(j).wait()

        att_epilogue()

        def b_body(i, c):
            ffn_block(i)

            @pl.when(li == N_LAYERS - 1)
            def _():
                out_copy(i).start()

            return c

        lax.fori_loop(0, nrb, b_body, 0)
        return carry

    lax.fori_loop(0, N_LAYERS, layer, 0)
    for i in range(nrb):
        out_copy(i).wait()


@jax.jit
def pallas_interleave_layers__softmax_full_mha__glu_gated_bilinear__prompt_kernel(
    A_x: jax.Array,
    A_wqkv: jax.Array,
    A_wo: jax.Array,
    B_x: jax.Array,
    B_w_gate: jax.Array,
    B_w_up: jax.Array,
    B_w_down: jax.Array,
):
    del B_x
    B, S, D = A_x.shape
    assert B == 1
    F = B_w_gate.shape[1]
    x2 = A_x.reshape(S, D)
    dh = D // N_HEADS

    scratch = [
        pltpu.VMEM((S, D), A_x.dtype),
        pltpu.VMEM(A_wqkv.shape, A_wqkv.dtype),
        pltpu.VMEM(A_wo.shape, A_wo.dtype),
        pltpu.VMEM(B_w_gate.shape, B_w_gate.dtype),
        pltpu.VMEM(B_w_up.shape, B_w_up.dtype),
        pltpu.VMEM(B_w_down.shape, B_w_down.dtype),
        pltpu.VMEM((S, D), F32),
        pltpu.VMEM((2 * S, D), BF16),
        pltpu.VMEM((S, D), BF16),
        pltpu.VMEM((D, S), BF16),
        pltpu.VMEM((D, S), BF16),
        pltpu.VMEM((D, S), F32),
        pltpu.VMEM((RB, F), BF16),
        pltpu.VMEM((S // 2, QB), F32),
        pltpu.VMEM((S // 2, QB), F32),
        pltpu.VMEM((S // 2, QB), F32),
        pltpu.VMEM((S // 2, QB), F32),
        pltpu.VMEM((2, 8, QB), F32),
        pltpu.VMEM((8, QB), F32),
        pltpu.VMEM((dh, QB), F32),
        pltpu.SMEM((2,), jnp.int32),
        pltpu.SemaphoreType.DMA((S // RB + 5,)),
    ]
    any_spec = pl.BlockSpec(memory_space=pl.ANY)
    out = pl.pallas_call(
        functools.partial(_kernel, S=S, D=D, F=F),
        out_shape=jax.ShapeDtypeStruct((S, D), A_x.dtype),
        in_specs=[any_spec] * 6,
        out_specs=any_spec,
        scratch_shapes=scratch,
        compiler_params=pltpu.CompilerParams(vmem_limit_bytes=100 * 1024 * 1024),
    )(x2, A_wqkv, A_wo, B_w_gate, B_w_up, B_w_down)
    return out.reshape(B, S, D)
```

```python
import functools
import math

import jax
import jax.numpy as jnp
from jax import lax
import jax.experimental.pallas as pl
import jax.experimental.pallas.tpu as pltpu

F32 = jnp.float32
BF16 = jnp.bfloat16

N_HEADS = 32
N_LAYERS = 2
LN_EPS = 1e-5
L_MIN, L_MAX = 2.0 ** -60, 2.0 ** 60
F32_MAX = float(jnp.finfo(jnp.float32).max)

QB = 512
CK = 128
SUB = 4
LAG = 6
SKEW = 2
RB = 512
RS = 128
RP = 64
PINS = (4, 6, 2, 5)
XSTEP = 8
NOFF = 16
OFFLOAD = tuple(-(-(k + 1) * 16 // NOFF) - 1 for k in range(NOFF))
_jobs = [(c, kg) for c in OFFLOAD for kg in (0, 1)]
VJOBS = [_jobs[c * len(_jobs) // 16:(c + 1) * len(_jobs) // 16] for c in range(16)]
FDELAY = 2
CHAIN = 2
BOFF = 4
RUNA = 2
PSTEP = 2
PBOTH = 0
VGRP = 0
PF32 = 0
QEXP = 0
GATHER = 1
PERM32 = (0, 1)
EPI = 2


def _layernorm(x):
    m = jnp.mean(x, axis=-1, keepdims=True)
    xc = x - m
    v = jnp.mean(xc * xc, axis=-1, keepdims=True)
    return xc * lax.rsqrt(v + LN_EPS)


U32 = jnp.uint32


def _pack(x):
    return pltpu.bitcast(x.astype(BF16), U32)


def _unpack(x):
    return pltpu.bitcast(x, BF16)


def _dot(a, b):
    return lax.dot_general(a, b, (((1,), (0,)), ((), ())), preferred_element_type=F32)


def _lhs_terms(a11, a12, a21, a22):
    return [a11 + a22, a21 + a22, a11, a22, a11 + a12, a21 - a11, a12 - a22]


def _rhs_terms(b11, b12, b21, b22):
    return [b11 + b22, b12 - b22, b21 - b11, b11 + b12, b21 + b22]


def _strassen(lhs, rhs):
    m1 = _dot(lhs(0), rhs(0))
    m4 = _dot(lhs(3), rhs(3))
    c11 = m1 + m4
    m2 = _dot(lhs(1), rhs(1))
    c21 = m2 + m4
    c22 = m1 - m2
    m5 = _dot(lhs(4), rhs(4))
    c11 = c11 - m5
    m7 = _dot(lhs(6), rhs(6))
    c11 = c11 + m7
    m3 = _dot(lhs(2), rhs(2))
    c12 = m3 + m5
    c22 = c22 + m3
    m6 = _dot(lhs(5), rhs(5))
    c22 = c22 + m6
    return c11, c12, c21, c22


_RHS_SLOT = {0: 0, 2: 1, 3: 2, 5: 3, 6: 4}


def _kernel(x_hbm, wqkv_hbm, wo_hbm, wg_hbm, wu_hbm, wd_hbm, out_hbm,
            xio, wqkv, wo, wg, wu, wd, cqkv, cg, cu, cd,
            x_ref, ln_ref, k_ref, qt_ref, vt_ref, ot_ref, h_ref,
            pc_ref, l_ref, bad_ref, oc_ref, qb_ref, qb1_ref, idx_ref, z_ref, sems, *, S, D, F):
    dh = D // N_HEADS
    gph = 128 // dh
    nt = N_HEADS // gph
    nqb = S // QB
    nc = S // CK
    half = nc // 2
    sr = CK // SUB
    nit = nt * nqb
    nrb = S // RB
    lagc = nc + SKEW
    qscale = (dh ** -0.5) * math.log2(math.e)
    hb, hd, hf = RB // 2, D // 2, F // 2

    def blk(i):
        return pl.ds(pl.multiple_of(i * RB, RB), RB)

    def x_copy(i):
        return pltpu.make_async_copy(x_hbm.at[blk(i), :], xio.at[blk(i), :], sems.at[i])

    def out_copy(i):
        return pltpu.make_async_copy(xio.at[blk(i), :], out_hbm.at[blk(i), :], sems.at[i])

    w_pairs = ((wqkv_hbm, wqkv), (wo_hbm, wo), (wg_hbm, wg), (wu_hbm, wu), (wd_hbm, wd))

    def w_copy(j):
        return pltpu.make_async_copy(w_pairs[j][0], w_pairs[j][1], sems.at[nrb + j])

    x_copy(0).start()
    w_copy(0).start()
    x_copy(1).start()

    def half_rows(r0, nr):
        if isinstance(r0, int):
            return pl.ds(r0 // 2, nr // 2)
        return pl.ds(pl.multiple_of(r0 // 2, 8), nr // 2)

    def ln_terms(xt, xb):
        lt, lb = _layernorm(xt), _layernorm(xb)
        terms = _lhs_terms(lt[:, :hd], lt[:, hd:], lb[:, :hd], lb[:, hd:])
        return _pack(jnp.concatenate(terms, axis=1))

    def weight_terms(w, c, r0, nr, kh, c0, nh):
        top, bot = pl.ds(r0, nr), pl.ds(r0 + kh, nr)
        terms = _rhs_terms(w[top, c0:c0 + nh].astype(F32), w[top, c0 + nh:c0 + 2 * nh].astype(F32),
                           w[bot, c0:c0 + nh].astype(F32), w[bot, c0 + nh:c0 + 2 * nh].astype(F32))
        for j, t in enumerate(terms):
            c[j, half_rows(r0, nr), c0 // 2:c0 // 2 + nh] = _pack(t)
        return terms

    def rhs_of(w, c, kh, c0, nh, n, nn):
        def rhs(i):
            if i == 1:
                return w[0:kh, c0 + n:c0 + n + nn]
            if i == 4:
                return w[kh:2 * kh, c0 + nh + n:c0 + nh + n + nn]
            return _unpack(c[_RHS_SLOT[i], :, c0 // 2 + n:c0 // 2 + n + nn])
        return rhs

    def ln_rows(which, b, r, n):
        return pl.ds(pl.multiple_of(((which * nrb + b) * hb + r) // 2, RP // 2), n // 2)

    def ln_piece(which, b, r, xt, xb):
        piece = ln_terms(xt, xb)
        ln_ref[ln_rows(which, b, r, xt.shape[0]), :] = piece
        return piece

    def x_rows(b, r):
        return pl.ds(pl.multiple_of(b * RB + r, RP), RP)

    z_ref[0] = 0
    z_ref[1] = 0
    idx_ref[...] = lax.broadcasted_iota(jnp.int32, idx_ref.shape, 0)
    pc_ref[...] = jnp.zeros_like(pc_ref)
    l_ref[...] = jnp.ones_like(l_ref)
    oc_ref[...] = jnp.zeros_like(oc_ref)
    x_copy(0).wait()
    x0 = xio[0:RB, :].astype(F32)
    ln_piece(1, 0, 0, x0[:hb], x0[hb:])
    w_copy(0).wait()
    for b in range(2, nrb):
        x_copy(b).start()
    for p in range(3):
        weight_terms(wqkv, cqkv, 0, hd, hd, p * D, hd)

    def lhs_of(z0, a, piece):
        def lhs(j):
            t = a[:, j * hd:(j + 1) * hd]
            if piece is not None and j in PINS:
                n = piece.shape[0]
                per = t.shape[0] // n
                k0 = PINS.index(j) * per
                parts = []
                for r in range(per):
                    tr = t[r * n:(r + 1) * n]
                    if k0 + r < 7:
                        tr = jnp.where(z0 == 0, tr, piece[:, (k0 + r) * hd:(k0 + r + 1) * hd])
                    parts.append(tr)
                t = jnp.concatenate(parts, axis=0)
            return _unpack(t)
        return lhs

    def resid(li, rows):
        return jnp.where(li == 0, xio[rows, :].astype(F32), x_ref[rows, :])

    def qkv_block(li, i):
        z0 = z_ref[0]
        a0 = ln_ref[ln_rows(1, i, 0, hb), :]
        nxt = jnp.minimum(i + 1, nrb - 1)
        todo = list(range(0, hb, 2 * RP))

        def proj(p):
            piece = None
            if p != 0:
                r = todo.pop(0)
                xs = []
                for rr in (r, hb + r):
                    rows = pl.ds(pl.multiple_of(nxt * RB + rr, 2 * RP), 2 * RP)
                    xs.append(resid(li, rows))
                piece = ln_piece(1, nxt, r, xs[0], xs[1])
            c11, c12, c21, c22 = _strassen(lhs_of(z0, a0, piece),
                                           rhs_of(wqkv, cqkv, hd, p * D, hd, 0, hd))
            return jnp.concatenate([jnp.concatenate([c11, c12], axis=1),
                                    jnp.concatenate([c21, c22], axis=1)], axis=0)

        rows = blk(i)
        qt_ref[:, rows] = _pack((proj(0) * qscale).T)
        vt_ref[:, rows] = _pack(proj(2).T)
        k_ref[half_rows(i * RB, RB), :] = _pack(proj(1))
        assert not todo

    def wo_pieces(li):
        order = [0, 2, 1, 3] + list(range(4, S // RS))
        keep = {}
        for r in order:
            rows = slice(r * RS, (r + 1) * RS)
            o = ot_ref[:, rows].T.astype(BF16)
            ys = []
            for n in range(0, D, 128):
                ys.append(_dot(o, wo[:, n:n + 128]))
                if n + 128 == D:
                    x = resid(li, rows) + jnp.concatenate(ys, axis=1)
                    x_ref[rows, :] = x
                    keep[r] = x
                    if r in (2, 3):
                        ln_piece(0, 0, (r - 2) * RS, keep[r - 2], x)
                yield

    def ffn_block(i):
        z0 = z_ref[0]
        nxt = jnp.minimum(i + 1, nrb - 1)
        todo = [(0, nxt, r) for r in range(0, hb, RP)]
        todo += [(1, 0, (i % 2) * (hb // 2) + r) for r in range(0, hb // 2, RP)]
        a0 = ln_ref[ln_rows(0, i, 0, hb), :]
        for n in range(0, hf, 128):
            piece = None
            if n > 0 and todo:
                which, b, r = todo.pop(0)
                piece = ln_piece(which, b, r, x_ref[x_rows(b, r), :], x_ref[x_rows(b, hb + r), :])
            rg = rhs_of(wg, cg, hd, 0, hf, n, 128)
            ru = rhs_of(wu, cu, hd, 0, hf, n, 128)
            cs = _strassen(lhs_of(z0, a0, piece),
                           lambda j: jnp.concatenate([rg(j), ru(j)], axis=1))
            hs = [c[:, :128] * c[:, 128:] for c in cs]
            for j, t in enumerate(_lhs_terms(*hs)):
                h_ref[j, :, n:n + 128] = _pack(t)
        assert not todo
        c11, c12, c21, c22 = _strassen(lambda j: _unpack(h_ref[j]), rhs_of(wd, cd, hf, 0, hd, 0, hd))
        rows = blk(i)
        y = x_ref[rows, :] + jnp.concatenate([jnp.concatenate([c11, c12], axis=1),
                                              jnp.concatenate([c21, c22], axis=1)], axis=0)
        x_ref[rows, :] = y
        xio[rows, :] = y.astype(xio.dtype)

    def head_row(it, g):
        return pl.multiple_of((it % nt) * 128 + g * dh, dh)

    def head_rows_packed(it, g):
        return pl.ds(pl.multiple_of((it % nt) * 64 + g * (dh // 2), dh // 2), dh // 2)

    def q_col(it):
        return pl.multiple_of((it // nt) * QB, QB)

    def wq(it, g):
        q = _unpack(qt_ref[head_rows_packed(it, g), pl.ds(q_col(it), QB)])
        parts = []
        if g > 0:
            parts.append(jnp.zeros((g * dh, QB), BF16))
        parts.append(q)
        if g < gph - 1:
            parts.append(jnp.zeros(((gph - 1 - g) * dh, QB), BF16))
        return jnp.concatenate(parts, axis=0)

    def q_bcast(it, g):
        qf = _unpack(qt_ref[head_rows_packed(it, g), pl.ds(q_col(it), QB)]).astype(F32)
        return [jnp.broadcast_to(qf[d:d + 1], (8, QB)) for d in range(dh)]

    def k_rows(it, r0, n):
        return _unpack(k_ref[r0 // 2:(r0 + n) // 2, pl.ds(pl.multiple_of((it % nt) * 128, 128), 128)])

    def k_group(it, r16):
        return k_ref[r16 * 8:(r16 + 1) * 8, pl.ds(pl.multiple_of((it % nt) * 128, 128), 128)]

    def pv_dot(it, g, t, pb, o):
        v = _unpack(vt_ref[head_rows_packed(it, g), t * CK:(t + 1) * CK])
        return o + _dot(v, pb)

    def pv_finish(it, g, l, o):
        lt = jnp.sum(l, axis=0, keepdims=True)
        res = o / lt
        ot_ref[pl.ds(head_row(it, g), dh), pl.ds(q_col(it), QB)] = res
        ok = (lt >= L_MIN) & (lt <= L_MAX)
        fin = jnp.abs(res) <= F32_MAX
        ok = fin[0:8] & fin[8:16] & ok
        return jnp.where(ok, 0.0, 1.0)

    gpt = CK // 16
    ntile = gph * nc

    def att_body(it, carry):
        z0 = z_ref[0]
        z1 = z_ref[1]
        prv = jnp.maximum(it - 1, 0)
        nxt = jnp.minimum(it + 1, nit - 1)
        nr = hd // nit
        r0 = pl.multiple_of(it * nr, nr)
        terms = weight_terms(wg, cg, r0, nr, hd, 0, hf) + weight_terms(wu, cu, r0, nr, hd, 0, hf)
        r0 = pl.multiple_of(jnp.minimum(it, hf // 64 - 1) * 64, 64)
        terms += weight_terms(wd, cd, r0, 64, hf, 0, hd)
        tiles = [t[r:r + 8, n:n + 128] for t in terms
                 for n in range(0, t.shape[1], 128) for r in range(0, t.shape[0], 8)]
        per = QB // 128
        extra = [jnp.concatenate(tiles[k:k + per], axis=1) for k in range(0, len(tiles), per)]

        stream = []
        for T in range(ntile):
            stream.append([(T, r) for r in range(gpt - 1, -1, -1)
                           if not (T % nc in OFFLOAD and r == VGRP)])
        pieces = []
        for T in range(ntile + 1):
            pc = stream[T - 1][-BOFF:] if T > 0 else []
            if T < ntile:
                pc = pc + stream[T][:-BOFF]
            pieces.append(pc)

        ws = {}
        qbs = (qb_ref, qb1_ref)
        qrows = {g: (lambda d, g=g: qbs[g % 2][z1 + d]) for g in range(gph)}
        pgroups = {}
        ls = {}
        pins = []
        st = {"acc": None}
        total = len(OFFLOAD) * dh
        ocs = []

        def consume(T, r, s):
            p = jnp.exp2(s)
            g = T // nc
            p2 = p[0:8] + p[8:16]
            ls[g] = p2 if g not in ls else ls[g] + p2
            pgroups[(T, r)] = p

        ngrp = gpt * nc - len(OFFLOAD)
        count = {}

        def vpu_slice(g):
            step = count[g] = count.get(g, -1) + 1
            for t_ in range(step * total // ngrp, (step + 1) * total // ngrp):
                oc, d = OFFLOAD[t_ // dh], t_ % dh
                if d == 0:
                    st["k"] = k_group(it, oc * gpt + VGRP)
                col = g * dh + d
                wide = (t_ % PERM32[1]) < PERM32[0]
                if GATHER:
                    idx = idx_ref[col]
                    if wide:
                        kf = _unpack(st["k"]).astype(F32)
                        kb = jnp.concatenate([jnp.take_along_axis(kf[0:8], idx, axis=1, mode="promise_in_bounds"),
                                              jnp.take_along_axis(kf[8:16], idx, axis=1, mode="promise_in_bounds")], axis=0)
                    else:
                        kb = _unpack(jnp.take_along_axis(st["k"], idx, axis=1, mode="promise_in_bounds")).astype(F32)
                elif wide:
                    kf = kf_ref[oc * 16:(oc + 1) * 16, pl.ds(pl.multiple_of((it % nt) * 128, 128), 128)]
                    kb = jnp.broadcast_to(kf[:, col:col + 1], (16, 128))
                else:
                    kb = _unpack(jnp.broadcast_to(st["k"][:, col:col + 1], (8, 128))).astype(F32)
                kb = jnp.concatenate([kb] * (QB // 128), axis=1).reshape(2, 8, QB)
                t = kb * qrows[g](d)[None]
                st["acc"] = t if d == 0 else st["acc"] + t
                if d == dh - 1:
                    consume(g * nc + oc, VGRP, st["acc"].reshape(16, QB))
            if step % PSTEP == PSTEP - 1 and st["acc"] is not None:
                return [st["acc"][0], st["acc"][1] if PBOTH else None]
            return [pins.pop(0) if pins else None, None]

        o = oc_ref[...]
        bad = bad_ref[...]
        for j in range(ntile + 1):
            if j < ntile and j % nc == 0:
                g = j // nc
                ws[g] = wq(it, g)
                qn = q_bcast(it, g + 1) if g < gph - 1 else q_bcast(nxt, 0)
                if not QEXP:
                    qrows[g + 1] = qn.__getitem__
            if j < ntile:
                pins.append(qn[j % nc])
                if QEXP or j // nc == gph - 1:
                    qbs[(j // nc + 1) % 2][z0 + j % nc] = qn[j % nc]
                if extra and j % 2 == 1:
                    pins.append(extra.pop(0))
            for g in sorted(set(T // nc for T, _ in pieces[j])):
                grp = [(T, r) for T, r in pieces[j] if T // nc == g]
                ks = [k_group(it, (T % nc) * gpt + r) for T, r in grp]
                if len(ocs) >= RUNA:
                    ks[0] = jnp.where(z1 == 0, ks[0], pltpu.bitcast(ocs[-RUNA][0:8, 0:128], U32))
                s = _dot(_unpack(jnp.concatenate(ks, axis=0)), ws[g])
                for k, (T, r) in enumerate(grp):
                    halves = [s[k * 16:k * 16 + 8], s[k * 16 + 8:k * 16 + 16]]
                    for hh, pin in enumerate(vpu_slice(g)):
                        if pin is not None:
                            halves[hh] = jnp.where(z0 == 0, halves[hh], pin)
                    consume(T, r, jnp.concatenate(halves, axis=0))
            T = j - 2
            if j >= ntile:
                break
            if T < 0:
                o = pv_dot(prv, gph - 1, nc + T, _unpack(pc_ref[j]), o)
                if T == -1:
                    bad = jnp.maximum(bad, pv_finish(prv, gph - 1, l_ref[...], o))
            else:
                g, t = T // nc, T % nc
                if t == 0:
                    o = jnp.where(z1 == 0, 0.0, o)
                pb = jnp.concatenate([pgroups.pop((T, r)) for r in range(gpt)], axis=0)
                o = pv_dot(it, g, t, pb if PF32 else pb.astype(BF16), o)
                if t == nc - 1:
                    bad = jnp.maximum(bad, pv_finish(it, g, ls[g], o))
            ocs.append(o)
        for k in range(2):
            T = ntile - 2 + k
            pc_ref[k] = _pack(jnp.concatenate([pgroups.pop((T, r)) for r in range(gpt)], axis=0))
        l_ref[...] = ls[gph - 1]
        oc_ref[...] = o
        bad_ref[...] = bad
        assert not extra and not pgroups
        return carry

    def att_tail():
        it = nit - 1
        o = oc_ref[...]
        for k in range(2):
            o = pv_dot(it, gph - 1, nc - 2 + k, _unpack(pc_ref[k]), o)
        bad = jnp.maximum(bad_ref[...], pv_finish(it, gph - 1, l_ref[...], o))
        return jnp.max(bad)

    def att_safe_body(u, carry):
        it, g = u // gph, u % gph
        tile = pl.multiple_of((it % nt) * 128, 128)
        cols = pl.ds(q_col(it), QB)
        qt = qt_ref[pl.ds(pl.multiple_of((it % nt) * 64, 64), 64), cols]
        grp = lax.broadcasted_iota(jnp.int32, qt.shape, 0) // (dh // 2)
        w = _unpack(jnp.where(grp == g, qt, jnp.zeros_like(qt)))
        s = _dot(_unpack(k_ref[:, pl.ds(tile, 128)]), w)
        p = jnp.exp2(s - jnp.max(s, axis=0, keepdims=True))
        lt = jnp.sum(p, axis=0, keepdims=True)
        o = _dot(_unpack(vt_ref[head_rows_packed(it, g), :]), p.astype(BF16))
        ot_ref[pl.ds(head_row(it, g), dh), cols] = o / lt
        return carry

    def layer(li, carry):
        def a_body(i, c):
            @pl.when(li == 0)
            def _():
                @pl.when(i + 1 < nrb)
                def _():
                    x_copy(i + 1).wait()

                @pl.when(i == 1)
                def _():
                    for j in range(1, 5):
                        w_copy(j).start()

            qkv_block(li, i)
            return c

        lax.fori_loop(0, nrb, a_body, 0)

        @pl.when(li == 0)
        def _():
            for j in range(1, 5):
                w_copy(j).wait()

        for d, q in enumerate(q_bcast(0, 0)):
            qb_ref[d] = q
        bad_ref[...] = jnp.zeros_like(bad_ref)
        lax.fori_loop(0, nit, att_body, 0)

        @pl.when(att_tail() > 0.5)
        def _():
            lax.fori_loop(0, nit * gph, att_safe_body, 0)

        for _ in wo_pieces(li):
            pass

        def b_body(i, c):
            ffn_block(i)

            @pl.when(li == N_LAYERS - 1)
            def _():
                out_copy(i).start()

            return c

        lax.fori_loop(0, nrb, b_body, 0)
        return carry

    lax.fori_loop(0, N_LAYERS, layer, 0)
    for i in range(nrb):
        out_copy(i).wait()


@jax.jit
def pallas_interleave_layers__softmax_full_mha__glu_gated_bilinear__prompt_kernel(
    A_x: jax.Array,
    A_wqkv: jax.Array,
    A_wo: jax.Array,
    B_x: jax.Array,
    B_w_gate: jax.Array,
    B_w_up: jax.Array,
    B_w_down: jax.Array,
):
    del B_x
    B, S, D = A_x.shape
    assert B == 1
    F = B_w_gate.shape[1]
    x2 = A_x.reshape(S, D)
    dh = D // N_HEADS

    scratch = [
        pltpu.VMEM((S, D), A_x.dtype),
        pltpu.VMEM(A_wqkv.shape, A_wqkv.dtype),
        pltpu.VMEM(A_wo.shape, A_wo.dtype),
        pltpu.VMEM(B_w_gate.shape, B_w_gate.dtype),
        pltpu.VMEM(B_w_up.shape, B_w_up.dtype),
        pltpu.VMEM(B_w_down.shape, B_w_down.dtype),
        pltpu.VMEM((5, D // 4, 3 * D // 2), U32),
        pltpu.VMEM((5, D // 4, F // 2), U32),
        pltpu.VMEM((5, D // 4, F // 2), U32),
        pltpu.VMEM((5, F // 4, D // 2), U32),
        pltpu.VMEM((S, D), F32),
        pltpu.VMEM((S // 2, 7 * D // 2), U32),
        pltpu.VMEM((S // 2, D), U32),
        pltpu.VMEM((D // 2, S), U32),
        pltpu.VMEM((D // 2, S), U32),
        pltpu.VMEM((D, S), F32),
        pltpu.VMEM((7, RB // 4, F // 2), U32),
        pltpu.VMEM((2, CK // 2, QB), U32),
        pltpu.VMEM((8, QB), F32),
        pltpu.VMEM((8, QB), F32),
        pltpu.VMEM((dh, QB), F32),
        pltpu.VMEM((dh, 8, QB), F32),
        pltpu.VMEM((dh, 8, QB), F32),
        pltpu.VMEM((128, 8, 128), jnp.int32),
        pltpu.SMEM((2,), jnp.int32),
        pltpu.SemaphoreType.DMA((S // RB + 5,)),
    ]
    any_spec = pl.BlockSpec(memory_space=pl.ANY)
    out = pl.pallas_call(
        functools.partial(_kernel, S=S, D=D, F=F),
        out_shape=jax.ShapeDtypeStruct((S, D), A_x.dtype),
        in_specs=[any_spec] * 6,
        out_specs=any_spec,
        scratch_shapes=scratch,
        compiler_params=pltpu.CompilerParams(vmem_limit_bytes=100 * 1024 * 1024),
    )(x2, A_wqkv, A_wo, B_w_gate, B_w_up, B_w_down)
    return out.reshape(B, S, D)
```

```python
import functools
import math

import jax
import jax.numpy as jnp
from jax import lax
import jax.experimental.pallas as pl
import jax.experimental.pallas.tpu as pltpu

F32 = jnp.float32
BF16 = jnp.bfloat16
U32 = jnp.uint32

N_HEADS = 32
N_LAYERS = 2
LN_EPS = 1e-5
L_MIN, L_MAX = 2.0 ** -60, 2.0 ** 60
F32_MAX = float(jnp.finfo(jnp.float32).max)

T = 128
QB = 512
RB = 512
BOFF = 4
RUNA = 2
PSTEP = 2
PINS = (4, 6, 2, 5)
XP = 2
FLAT = 1
RP1 = 64
RP2 = 16
FP1 = (592, 5)
FP2 = (606, 5)
FPN = 24
WOP = 8
MSPLIT = 2
FDEL = 3
FPIN0 = 14


def _layernorm(x):
    m = jnp.mean(x, axis=-1, keepdims=True)
    xc = x - m
    v = jnp.mean(xc * xc, axis=-1, keepdims=True)
    return xc * lax.rsqrt(v + LN_EPS)


def _pack(x):
    return pltpu.bitcast(x.astype(BF16), U32)


def _unpack(x):
    return pltpu.bitcast(x, BF16)


def _dot(a, b):
    return lax.dot_general(a, b, (((1,), (0,)), ((), ())), preferred_element_type=F32)


def _block(g):
    return jnp.concatenate([jnp.concatenate(r, axis=1) for r in g], axis=0)


class _G:
    def __init__(self, g):
        self.g = g

    def __add__(self, o):
        return _G([[a + b for a, b in zip(r, s)] for r, s in zip(self.g, o.g)])

    def __sub__(self, o):
        return _G([[a - b for a, b in zip(r, s)] for r, s in zip(self.g, o.g)])

    def flat(self):
        return self.g[0] + self.g[1]


def _lhs_terms(a11, a12, a21, a22):
    return [a11 + a22, a21 + a22, a11, a22, a11 + a12, a21 - a11, a12 - a22]


def _rhs_terms(b11, b12, b21, b22):
    return [b11 + b22, b11, b12 - b22, b21 - b11, b22, b11 + b12, b21 + b22]


def _quads(g4):
    return [_G([r[2 * c:2 * c + 2] for r in g4[2 * k:2 * k + 2]]) for k in range(2) for c in range(2)]


def _terms2(fn, g4):
    outer = fn(*_quads(g4))
    return outer, [t for o in outer for t in fn(*o.flat())]


_ORDER = (0, 3, 1, 4, 6, 2, 5)


def _strassen(prod):
    m = {i: None for i in range(7)}
    m[0] = prod(0)
    m[3] = prod(3)
    c11 = m[0] + m[3]
    m[1] = prod(1)
    c21 = m[1] + m[3]
    c22 = m[0] - m[1]
    m[4] = prod(4)
    c11 = c11 - m[4]
    c11 = c11 + prod(6)
    m[2] = prod(2)
    c12 = m[2] + m[4]
    c22 = c22 + m[2]
    c22 = c22 + prod(5)
    return [[c11, c12], [c21, c22]]


def _strassen2(prod):
    c = _strassen(lambda i: _G(_strassen(lambda j: prod(i, j))))
    return [c[r // 2][0].g[r % 2] + c[r // 2][1].g[r % 2] for r in range(4)]


_COEF = ({0: 1, 3: 1, 4: -1, 6: 1}, {2: 1, 4: 1}, {1: 1, 3: 1}, {0: 1, 1: -1, 2: 1, 5: 1})


def _strassen2_flat(prod):
    p = {(i, j): prod(i, j) for i in _ORDER for j in _ORDER}
    out = [[None] * 4 for _ in range(4)]
    for q1 in range(4):
        for q2 in range(4):
            pos = [p[k] for k in p if _COEF[q1].get(k[0], 0) * _COEF[q2].get(k[1], 0) > 0]
            neg = [p[k] for k in p if _COEF[q1].get(k[0], 0) * _COEF[q2].get(k[1], 0) < 0]
            acc = pos[0]
            for t in neg:
                acc = acc - t
            for t in pos[1:]:
                acc = acc + t
            out[2 * (q1 // 2) + q2 // 2][2 * (q1 % 2) + q2 % 2] = acc
    return out


def _kernel(x_hbm, wqkv_hbm, wo_hbm, wg_hbm, wu_hbm, wd_hbm, out_hbm,
            xio, wqkv, wo, wgu, wd, cqkv, c2gu, c1gu, c2d, c1d,
            x_ref, xm_ref, ln1_ref, ln2_ref, k_ref, qt_ref, vt_ref, ot_ref,
            pc_ref, l_ref, bad_ref, oc_ref, qb_ref, idx_ref, z_ref, sems, *, S, D, F):
    dh = D // N_HEADS
    gph = T // dh
    nt = N_HEADS // gph
    nqb = S // QB
    nc = S // T
    nit = nt * nqb
    nrb = S // RB
    qscale = (dh ** -0.5) * math.log2(math.e)
    hb, hd = RB // 2, D // 2
    qb4 = RB // 4
    fq = (F // T) // 4
    fm = 4 * fq * T
    assert D == 4 * T and qb4 == T and F - fm == 2 * T

    def blk(i):
        return pl.ds(pl.multiple_of(i * RB, RB), RB)

    def x_copy(i):
        return pltpu.make_async_copy(x_hbm.at[blk(i), :], xio.at[blk(i), :], sems.at[i])

    def out_copy(i):
        return pltpu.make_async_copy(xio.at[blk(i), :], out_hbm.at[blk(i), :], sems.at[i])

    w_pairs = ((wqkv_hbm, wqkv), (wo_hbm, wo), (wg_hbm, wgu.at[0]), (wu_hbm, wgu.at[1]), (wd_hbm, wd))

    def w_copy(j):
        return pltpu.make_async_copy(w_pairs[j][0], w_pairs[j][1], sems.at[nrb + j])

    x_copy(0).start()
    w_copy(0).start()
    x_copy(1).start()

    def rows(r0, n, mult):
        return pl.ds(r0, n) if isinstance(r0, int) else pl.ds(pl.multiple_of(r0, mult), n)

    def grid_terms(w, c, n, r0, nr, row0, rstep, col0, cw):
        g = [[w[rows(row0 + k * rstep + r0, nr, 16), col0 + j * cw:col0 + (j + 1) * cw].astype(F32)
              for j in range(n)] for k in range(n)]
        terms = _rhs_terms(*(g[0] + g[1])) if n == 2 else _terms2(_rhs_terms, g)[1]
        for j, t in enumerate(terms):
            c[j, rows(r0 // 2, nr // 2, 8), :] = _pack(t)
        return terms

    def ln1_piece(b, r, xt, xb):
        lt, lb = _layernorm(xt), _layernorm(xb)
        piece = _pack(jnp.concatenate(_lhs_terms(lt[:, :hd], lt[:, hd:], lb[:, :hd], lb[:, hd:]), axis=1))
        ln1_ref[rows((b * hb + r) // 2, xt.shape[0] // 2, 8), :] = piece
        return piece

    def ln2_piece(b, r, xs):
        ls = [_layernorm(x) for x in xs]
        outer, leaves = _terms2(_lhs_terms, [[l[:, c * T:(c + 1) * T] for c in range(4)] for l in ls])
        offd = [o.g[k][1 - k] for o in outer for k in range(2)]
        piece = _pack(jnp.concatenate(leaves + offd, axis=1))
        ln2_ref[rows((b * qb4 + r) // 2, xs[0].shape[0] // 2, 8), :] = piece
        return piece

    z_ref[0] = 0
    z_ref[1] = 0
    idx_ref[...] = lax.broadcasted_iota(jnp.int32, idx_ref.shape, 0)
    pc_ref[...] = jnp.zeros_like(pc_ref)
    l_ref[...] = jnp.ones_like(l_ref)
    oc_ref[...] = jnp.zeros_like(oc_ref)
    x_ref[...] = jnp.zeros_like(x_ref)
    x_copy(0).wait()
    x0 = xio[0:RB, :].astype(F32)
    ln1_piece(0, 0, x0[:hb], x0[hb:])
    w_copy(0).wait()
    for b in range(2, nrb):
        x_copy(b).start()
    for p in range(3):
        grid_terms(wqkv, cqkv.at[p], 2, 0, hd, 0, hd, p * D, hd)

    def pin_rows(z0, t, blocks):
        n = blocks[0].shape[0]
        parts = [jnp.where(z0 == 0, t[r * n:(r + 1) * n], b) for r, b in enumerate(blocks)]
        if len(blocks) * n < t.shape[0]:
            parts.append(t[len(blocks) * n:])
        return jnp.concatenate(parts, axis=0)

    def resid(li, rws):
        return jnp.where(li == 0, xio[rws, :].astype(F32), x_ref[rws, :])

    def qkv_block(li, i):
        z0 = z_ref[0]
        a0 = ln1_ref[rows(i * (hb // 2), hb // 2, 8), :]
        nxt = jnp.minimum(i + 1, nrb - 1)
        todo = list(range(0, hb, T))

        def proj(p):
            piece = None
            if p != 0:
                r = todo.pop(0)
                piece = ln1_piece(nxt, r, resid(li, rows(nxt * RB + r, T, T)),
                                  resid(li, rows(nxt * RB + hb + r, T, T)))

            def prod(j):
                t = a0[:, j * hd:(j + 1) * hd]
                if piece is not None and j in PINS:
                    k0 = PINS.index(j) * 2
                    t = pin_rows(z0, t, [piece[:, k * hd:(k + 1) * hd] for k in range(k0, min(k0 + 2, 7))])
                return _dot(_unpack(t), _unpack(cqkv[p, j]))

            return _block(_strassen(prod))

        qt_ref[:, blk(i)] = _pack((proj(0) * qscale).T)
        vt_ref[:, blk(i)] = _pack(proj(2).T)
        k_ref[rows(i * hb, hb, 8), :] = _pack(proj(1))
        assert not todo

    def tiles_of(pc):
        return [pc[h:h + 8, k:k + T] for k in range(0, pc.shape[1], T) for h in range(0, pc.shape[0], 8)]

    def wo_phase(li):
        z0 = z_ref[0]
        keep = []
        for r in range(S // T):
            rws = slice(r * T, (r + 1) * T)
            ot = ot_ref[:, rws]
            k = r - WOP
            if 0 <= k < qb4 // RP2:
                pc = ln2_piece(0, k * RP2, [x[k * RP2:(k + 1) * RP2] for x in keep[:4]])
                ot = pin_rows(z0, ot, [pltpu.bitcast(t, F32) for t in tiles_of(pc)])
            x = resid(li, rws) + _dot(ot.T.astype(BF16), wo[...])
            xm_ref[rws, :] = x
            keep.append(x)

    def ffn_block(i):
        z0 = z_ref[0]
        nxt = jnp.minimum(i + 1, nrb - 1)
        a0 = ln2_ref[rows(i * (qb4 // 2), qb4 // 2, 8), :]

        def a_blk(k):
            return a0[:, k * T:(k + 1) * T]

        side = []

        for n, r in enumerate(range(0, hb // 2, RP1)):
            r = (i % 2) * (hb // 2) + r
            pc = ln1_piece(0, r, x_ref[rows(r, RP1, RP1), :], x_ref[rows(hb + r, RP1, RP1), :])
            side.append((FP1[0] + n * FP1[1], tiles_of(pc)))
        for n, r in enumerate(range(0, qb4, RP2)):
            pc = ln2_piece(nxt, r, [xm_ref[rows(nxt * RB + q * qb4 + r, RP2, RP2), :] for q in range(4)])
            side.append((FP2[0] + n * FP2[1], tiles_of(pc)))
        seq = {"n": 0}

        def pinned(w):
            n = seq["n"] = seq["n"] + 1
            for start, pc in side:
                if pc and n > start:
                    return pin_rows(z0, w, [pc.pop(0) for _ in range(min(w.shape[0] // 8, FPN, len(pc)))])
            return w

        hterms = [[] for _ in range(49)]
        mr = T // 2 // MSPLIT
        for j in range(fq):
            def part(hf_, mat):
                def inner(i1):
                    def prod(i2):
                        k = i1 * 7 + i2
                        a = a_blk(k)[hf_ * mr:(hf_ + 1) * mr]
                        w = pinned(c2gu[mat, k, :, j * T:(j + 1) * T])
                        return _dot(_unpack(a), _unpack(w))

                    return _G(_strassen(prod))

                c = _strassen(inner)
                return [c[r // 2][0].g[r % 2] + c[r // 2][1].g[r % 2] for r in range(4)]

            hs = []
            for hf_ in range(MSPLIT):
                cg, cu = part(hf_, 0), part(hf_, 1)
                hs.append([[a * b for a, b in zip(r, q)] for r, q in zip(cg, cu)])
            h = [[jnp.concatenate([hh[r][c] for hh in hs], axis=0) for c in range(4)] for r in range(4)]
            for k, t in enumerate(_terms2(_lhs_terms, h)[1]):
                hterms[k].append(t)

        def prod1(i1):
            a = _block([[a_blk(i1 * 7 + 2), a_blk(49 + 2 * i1)], [a_blk(50 + 2 * i1), a_blk(i1 * 7 + 3)]])
            w = jnp.concatenate([pinned(c1gu[0, i1]), pinned(c1gu[1, i1])], axis=1)
            return _dot(_unpack(a), _unpack(w))

        c = _strassen(prod1)
        hrem = [t.astype(BF16) for t in _lhs_terms(*[b[:, :T] * b[:, T:] for r in c for b in r])]

        def down(i1):
            rem = _dot(hrem[i1], _unpack(c1d[i1]))
            m = _strassen(lambda i2: _dot(jnp.concatenate(hterms[i1 * 7 + i2], axis=1).astype(BF16),
                                          _unpack(pinned(c2d[i1 * 7 + i2]))))
            return rem + _block(m)

        y = xm_ref[blk(i), :] + _block(_strassen(down))
        assert not any(pc for _, pc in side)
        x_ref[blk(i), :] = y
        xio[blk(i), :] = y.astype(xio.dtype)

    def head_row(it, g):
        return pl.multiple_of((it % nt) * T + g * dh, dh)

    def head_rows_packed(it, g):
        return pl.ds(pl.multiple_of((it % nt) * (T // 2) + g * (dh // 2), dh // 2), dh // 2)

    def q_col(it):
        return pl.multiple_of((it // nt) * QB, QB)

    def wq(it, g):
        q = _unpack(qt_ref[head_rows_packed(it, g), pl.ds(q_col(it), QB)])
        parts = []
        if g > 0:
            parts.append(jnp.zeros((g * dh, QB), BF16))
        parts.append(q)
        if g < gph - 1:
            parts.append(jnp.zeros(((gph - 1 - g) * dh, QB), BF16))
        return jnp.concatenate(parts, axis=0)

    def q_bcast(it, g):
        qf = _unpack(qt_ref[head_rows_packed(it, g), pl.ds(q_col(it), QB)]).astype(F32)
        return [jnp.broadcast_to(qf[d:d + 1], (8, QB)) for d in range(dh)]

    def k_group(it, r16):
        return k_ref[r16 * 8:(r16 + 1) * 8, pl.ds(pl.multiple_of((it % nt) * T, T), T)]

    def pv_dot(it, g, t, pb, o):
        v = _unpack(vt_ref[head_rows_packed(it, g), t * T:(t + 1) * T])
        return o + _dot(v, pb)

    def pv_finish(it, g, l, o):
        lt = jnp.sum(l, axis=0, keepdims=True)
        res = o / lt
        ot_ref[pl.ds(head_row(it, g), dh), pl.ds(q_col(it), QB)] = res
        ok = (lt >= L_MIN) & (lt <= L_MAX)
        fin = jnp.abs(res) <= F32_MAX
        ok = fin[0:8] & fin[8:16] & ok
        return jnp.where(ok, 0.0, 1.0)

    gpt = T // 16
    ntile = gph * nc

    def ffn_weight_slice(it):
        m, k = it // 8, it % 8
        terms = grid_terms(wgu.at[m], c2gu.at[m], 4, k * 16, 16, 0, T, 0, fq * T)
        terms += grid_terms(wgu.at[m], c1gu.at[m], 2, k * 32, 32, 0, hd, fm, T)
        terms += grid_terms(wd, c2d, 4, jnp.minimum(it, fq * T // 32 - 1) * 32, 32, 0, fq * T, 0, T)
        terms += grid_terms(wd, c1d, 2, k * 16, 16, fm, T, 0, hd)
        return terms

    def att_body(it, carry):
        z0 = z_ref[0]
        z1 = z_ref[1]
        prv = jnp.maximum(it - 1, 0)
        nxt = jnp.minimum(it + 1, nit - 1)
        tiles = [t[r:r + 8, n:n + T] for t in ffn_weight_slice(it)
                 for n in range(0, t.shape[1], T) for r in range(0, t.shape[0], 8)]
        per = QB // T
        tiles += [tiles[-1]] * (-len(tiles) % per)
        extra = [jnp.concatenate(tiles[k:k + per], axis=1) for k in range(0, len(tiles), per)]

        stream = [[(t, r) for r in range(gpt - 1, 0, -1)] for t in range(ntile)]
        pieces = []
        for t in range(ntile + 1):
            pc = stream[t - 1][-BOFF:] if t > 0 else []
            if t < ntile:
                pc = pc + stream[t][:-BOFF]
            pieces.append(pc)

        ws = {}
        qrows = {0: lambda d: qb_ref[d]}
        pgroups = {}
        ls = {}
        pins = []
        st = {"acc": None}
        total = nc * dh
        ngrp = (gpt - 1) * nc
        count = {}
        ocs = []

        def consume(t, r, s):
            p = jnp.exp2(s)
            g = t // nc
            p2 = p[0:8] + p[8:16]
            ls[g] = p2 if g not in ls else ls[g] + p2
            pgroups[(t, r)] = p

        def vpu_slice(g):
            step = count[g] = count.get(g, -1) + 1
            for t_ in range(step * total // ngrp, (step + 1) * total // ngrp):
                oc, d = t_ // dh, t_ % dh
                if d == 0:
                    st["k"] = k_group(it, oc * gpt)
                kb = jnp.take_along_axis(st["k"], idx_ref[g * dh + d], axis=1, mode="promise_in_bounds")
                kb = _unpack(kb).astype(F32)
                kb = jnp.concatenate([kb] * (QB // T), axis=1).reshape(2, 8, QB)
                t = kb * qrows[g](d)[None]
                st["acc"] = t if d == 0 else st["acc"] + t
                if d == dh - 1:
                    consume(g * nc + oc, 0, st["acc"].reshape(16, QB))
            if step % PSTEP == PSTEP - 1:
                return st["acc"][0]
            return pins.pop(0) if pins else None

        o = oc_ref[...]
        bad = bad_ref[...]
        for j in range(ntile + 1):
            if j < ntile and j % nc == 0:
                g = j // nc
                ws[g] = wq(it, g)
                qn = q_bcast(it, g + 1) if g < gph - 1 else q_bcast(nxt, 0)
                qrows[g + 1] = qn.__getitem__
            if j < ntile:
                pins.append(qn[j % nc])
                if j // nc == gph - 1:
                    qb_ref[j % nc] = qn[j % nc]
                for _ in range(XP if j % 8 == 0 else 1):
                    if extra:
                        pins.append(extra.pop(0))
            for g in sorted(set(t // nc for t, _ in pieces[j])):
                grp = [(t, r) for t, r in pieces[j] if t // nc == g]
                ks = [k_group(it, (t % nc) * gpt + r) for t, r in grp]
                if len(ocs) >= RUNA:
                    ks[0] = jnp.where(z1 == 0, ks[0], pltpu.bitcast(ocs[-RUNA][0:8, 0:T], U32))
                s = _dot(_unpack(jnp.concatenate(ks, axis=0)), ws[g])
                for k, (t, r) in enumerate(grp):
                    sk = s[k * 16:(k + 1) * 16]
                    pin = vpu_slice(g)
                    if pin is not None:
                        sk = pin_rows(z0, sk, [pin])
                    consume(t, r, sk)
            if j >= ntile:
                break
            t = j - 2
            if t < 0:
                o = pv_dot(prv, gph - 1, nc + t, _unpack(pc_ref[j]), o)
                if t == -1:
                    bad = jnp.maximum(bad, pv_finish(prv, gph - 1, l_ref[...], o))
            else:
                g = t // nc
                if t % nc == 0:
                    o = jnp.where(z1 == 0, 0.0, o)
                pb = jnp.concatenate([pgroups.pop((t, r)) for r in range(gpt)], axis=0)
                o = pv_dot(it, g, t % nc, pb, o)
                if t % nc == nc - 1:
                    bad = jnp.maximum(bad, pv_finish(it, g, ls[g], o))
            ocs.append(o)
        for k in range(2):
            t = ntile - 2 + k
            pc_ref[k] = _pack(jnp.concatenate([pgroups.pop((t, r)) for r in range(gpt)], axis=0))
        l_ref[...] = ls[gph - 1]
        oc_ref[...] = o
        bad_ref[...] = bad
        assert not extra and not pgroups
        return carry

    def att_tail():
        it = nit - 1
        o = oc_ref[...]
        for k in range(2):
            o = pv_dot(it, gph - 1, nc - 2 + k, _unpack(pc_ref[k]), o)
        bad = jnp.maximum(bad_ref[...], pv_finish(it, gph - 1, l_ref[...], o))
        return jnp.max(bad)

    def att_safe_body(u, carry):
        it, g = u // gph, u % gph
        tile = pl.multiple_of((it % nt) * T, T)
        cols = pl.ds(q_col(it), QB)
        qt = qt_ref[pl.ds(pl.multiple_of((it % nt) * (T // 2), T // 2), T // 2), cols]
        grp = lax.broadcasted_iota(jnp.int32, qt.shape, 0) // (dh // 2)
        w = _unpack(jnp.where(grp == g, qt, jnp.zeros_like(qt)))
        s = _dot(_unpack(k_ref[:, pl.ds(tile, T)]), w)
        p = jnp.exp2(s - jnp.max(s, axis=0, keepdims=True))
        lt = jnp.sum(p, axis=0, keepdims=True)
        o = _dot(_unpack(vt_ref[head_rows_packed(it, g), :]), p.astype(BF16))
        ot_ref[pl.ds(head_row(it, g), dh), cols] = o / lt
        return carry

    def layer(li, carry):
        def a_body(i, c):
            @pl.when(li == 0)
            def _():
                @pl.when(i + 1 < nrb)
                def _():
                    x_copy(i + 1).wait()

                @pl.when(i == 1)
                def _():
                    for j in range(1, 5):
                        w_copy(j).start()

            qkv_block(li, i)
            return c

        lax.fori_loop(0, nrb, a_body, 0)

        @pl.when(li == 0)
        def _():
            for j in range(1, 5):
                w_copy(j).wait()

        for d, q in enumerate(q_bcast(0, 0)):
            qb_ref[d] = q
        bad_ref[...] = jnp.zeros_like(bad_ref)
        lax.fori_loop(0, nit, att_body, 0)

        @pl.when(att_tail() > 0.5)
        def _():
            lax.fori_loop(0, nit * gph, att_safe_body, 0)

        wo_phase(li)

        def b_body(i, c):
            ffn_block(i)

            @pl.when(li == N_LAYERS - 1)
            def _():
                out_copy(i).start()

            return c

        lax.fori_loop(0, nrb, b_body, 0)
        return carry

    lax.fori_loop(0, N_LAYERS, layer, 0)
    for i in range(nrb):
        out_copy(i).wait()


@jax.jit
def pallas_interleave_layers__softmax_full_mha__glu_gated_bilinear__prompt_kernel(
    A_x: jax.Array,
    A_wqkv: jax.Array,
    A_wo: jax.Array,
    B_x: jax.Array,
    B_w_gate: jax.Array,
    B_w_up: jax.Array,
    B_w_down: jax.Array,
):
    del B_x
    B, S, D = A_x.shape
    assert B == 1
    F = B_w_gate.shape[1]
    x2 = A_x.reshape(S, D)
    dh = D // N_HEADS
    fq = (F // T) // 4

    scratch = [
        pltpu.VMEM((S, D), A_x.dtype),
        pltpu.VMEM(A_wqkv.shape, A_wqkv.dtype),
        pltpu.VMEM(A_wo.shape, A_wo.dtype),
        pltpu.VMEM((2,) + B_w_gate.shape, B_w_gate.dtype),
        pltpu.VMEM(B_w_down.shape, B_w_down.dtype),
        pltpu.VMEM((3, 7, D // 4, D // 2), U32),
        pltpu.VMEM((2, 49, T // 2, fq * T), U32),
        pltpu.VMEM((2, 7, D // 4, T), U32),
        pltpu.VMEM((49, fq * T // 2, T), U32),
        pltpu.VMEM((7, T // 2, D // 2), U32),
        pltpu.VMEM((S, D), F32),
        pltpu.VMEM((S, D), F32),
        pltpu.VMEM((S // 4, 7 * D // 2), U32),
        pltpu.VMEM((S // 8, 63 * T), U32),
        pltpu.VMEM((S // 2, D), U32),
        pltpu.VMEM((D // 2, S), U32),
        pltpu.VMEM((D // 2, S), U32),
        pltpu.VMEM((D, S), F32),
        pltpu.VMEM((2, T // 2, QB), U32),
        pltpu.VMEM((8, QB), F32),
        pltpu.VMEM((8, QB), F32),
        pltpu.VMEM((dh, QB), F32),
        pltpu.VMEM((dh, 8, QB), F32),
        pltpu.VMEM((T, 8, T), jnp.int32),
        pltpu.SMEM((2,), jnp.int32),
        pltpu.SemaphoreType.DMA((S // RB + 5,)),
    ]
    any_spec = pl.BlockSpec(memory_space=pl.ANY)
    out = pl.pallas_call(
        functools.partial(_kernel, S=S, D=D, F=F),
        out_shape=jax.ShapeDtypeStruct((S, D), A_x.dtype),
        in_specs=[any_spec] * 6,
        out_specs=any_spec,
        scratch_shapes=scratch,
        compiler_params=pltpu.CompilerParams(vmem_limit_bytes=100 * 1024 * 1024),
    )(x2, A_wqkv, A_wo, B_w_gate, B_w_up, B_w_down)
    return out.reshape(B, S, D)
```

```python
import functools
import math

import jax
import jax.numpy as jnp
from jax import lax
import jax.experimental.pallas as pl
import jax.experimental.pallas.tpu as pltpu

F32 = jnp.float32
BF16 = jnp.bfloat16
U32 = jnp.uint32

N_HEADS = 32
N_LAYERS = 2
LN_EPS = 1e-5
L_MIN, L_MAX = 2.0 ** -60, 2.0 ** 60
F32_MAX = float(jnp.finfo(jnp.float32).max)

T = 128
QB = 512
RB = 512
BOFF = 4
RUNA = 3
PSTEP = 2
PINS = (4, 6, 2, 5)
XP = 2
RP1 = 64
RP2 = 16
FP1 = (592, 5)
FP2 = (604, 5)
FPN = 24
WOP = 11
MSPLIT = 2


def _layernorm(x):
    m = jnp.mean(x, axis=-1, keepdims=True)
    xc = x - m
    v = jnp.mean(xc * xc, axis=-1, keepdims=True)
    return xc * lax.rsqrt(v + LN_EPS)


def _pack(x):
    return pltpu.bitcast(x.astype(BF16), U32)


def _unpack(x):
    return pltpu.bitcast(x, BF16)


def _pack_pair(a, b):
    lo = pltpu.bitcast(b.astype(BF16).astype(F32), jnp.int32)
    lo = lax.shift_right_logical(lo, 16)
    bits = pltpu.bitcast(a, jnp.int32)
    mag = jnp.maximum((bits & 0x7FFFFFFF) - lo + 0x8000, 0) & 0x7FFF0000
    return (bits & jnp.int32(-2 ** 31)) | mag | lo


def _dot(a, b):
    return lax.dot_general(a, b, (((1,), (0,)), ((), ())), preferred_element_type=F32)


def _block(g):
    return jnp.concatenate([jnp.concatenate(r, axis=1) for r in g], axis=0)


class _G:
    def __init__(self, g):
        self.g = g

    def __add__(self, o):
        return _G([[a + b for a, b in zip(r, s)] for r, s in zip(self.g, o.g)])

    def __sub__(self, o):
        return _G([[a - b for a, b in zip(r, s)] for r, s in zip(self.g, o.g)])

    def flat(self):
        return self.g[0] + self.g[1]


def _lhs_terms(a11, a12, a21, a22):
    return [a11 + a22, a21 + a22, a11, a22, a11 + a12, a21 - a11, a12 - a22]


def _rhs_terms(b11, b12, b21, b22):
    return [b11 + b22, b11, b12 - b22, b21 - b11, b22, b11 + b12, b21 + b22]


def _quads(g4):
    return [_G([r[2 * c:2 * c + 2] for r in g4[2 * k:2 * k + 2]]) for k in range(2) for c in range(2)]


def _terms2(fn, g4):
    outer = fn(*_quads(g4))
    return outer, [t for o in outer for t in fn(*o.flat())]


def _strassen(prod):
    m = {i: None for i in range(7)}
    m[0] = prod(0)
    m[3] = prod(3)
    c11 = m[0] + m[3]
    m[1] = prod(1)
    c21 = m[1] + m[3]
    c22 = m[0] - m[1]
    m[4] = prod(4)
    c11 = c11 - m[4]
    c11 = c11 + prod(6)
    m[2] = prod(2)
    c12 = m[2] + m[4]
    c22 = c22 + m[2]
    c22 = c22 + prod(5)
    return [[c11, c12], [c21, c22]]


def _kernel(x_hbm, wqkv_hbm, wo_hbm, wg_hbm, wu_hbm, wd_hbm, out_hbm,
            xio, wqkv, wo, wgu, wd, cqkv, co, c2gu, c1gu, c2d, c1d,
            x_ref, xm_ref, ln1_ref, ln2_ref, k_ref, kv_ref, qt_ref, vt_ref, ot_ref,
            pc_ref, l_ref, bad_ref, oc_ref, qb_ref, idx_ref, z_ref, sems, *, S, D, F):
    dh = D // N_HEADS
    gph = T // dh
    nt = N_HEADS // gph
    nqb = S // QB
    nc = S // T
    nit = nt * nqb
    nrb = S // RB
    qscale = (dh ** -0.5) * math.log2(math.e)
    hb, hd = RB // 2, D // 2
    qb4 = RB // 4
    fq = (F // T) // 4
    fm = 4 * fq * T
    assert D == 4 * T and qb4 == T and F - fm == 2 * T and nrb == 4 and nit == 16

    def blk(i):
        return pl.ds(i * RB, RB) if isinstance(i, int) else pl.ds(pl.multiple_of(i * RB, RB), RB)

    def x_copy(i):
        return pltpu.make_async_copy(x_hbm.at[blk(i), :], xio.at[blk(i), :], sems.at[i])

    def out_copy(i, r, c):
        rws = pl.ds(i * RB + r * hb, hb) if isinstance(i, int) else pl.ds(pl.multiple_of(i * RB + r * hb, hb), hb)
        cols = pl.ds(c * hd, hd)
        return pltpu.make_async_copy(xio.at[rws, cols], out_hbm.at[rws, cols], sems.at[i])

    w_pairs = ((wo_hbm, wo), (wg_hbm, wgu.at[0]), (wu_hbm, wgu.at[1]), (wd_hbm, wd))

    def w_copy(j):
        return pltpu.make_async_copy(w_pairs[j][0], w_pairs[j][1], sems.at[nrb + 3 + j])

    def wqkv_copy(p):
        cols = pl.ds(p * D, D)
        return pltpu.make_async_copy(wqkv_hbm.at[:, cols], wqkv.at[:, cols], sems.at[nrb + p])

    x_copy(0).start()
    for p in (0, 2, 1):
        wqkv_copy(p).start()
    for b in range(1, nrb):
        x_copy(b).start()
    for j in (1, 2, 3, 0):
        w_copy(j).start()

    def rows(r0, n, mult):
        return pl.ds(r0, n) if isinstance(r0, int) else pl.ds(pl.multiple_of(r0, mult), n)

    def grid_terms(w, c, n, r0, nr, row0, rstep, col0, cw):
        g = [[w[rows(row0 + k * rstep + r0, nr, 16), col0 + j * cw:col0 + (j + 1) * cw].astype(F32)
              for j in range(n)] for k in range(n)]
        terms = _rhs_terms(*(g[0] + g[1])) if n == 2 else _terms2(_rhs_terms, g)[1]
        for j, t in enumerate(terms):
            c[j, rows(r0 // 2, nr // 2, 8), :] = _pack(t)
        return terms

    def ln1_piece(b, r, xt, xb):
        lt, lb = _layernorm(xt), _layernorm(xb)
        piece = _pack(jnp.concatenate(_lhs_terms(lt[:, :hd], lt[:, hd:], lb[:, :hd], lb[:, hd:]), axis=1))
        ln1_ref[rows((b * hb + r) // 2, xt.shape[0] // 2, 8), :] = piece
        return piece

    def ln2_piece(b, r, xs):
        ls = [_layernorm(x) for x in xs]
        outer, leaves = _terms2(_lhs_terms, [[l[:, c * T:(c + 1) * T] for c in range(4)] for l in ls])
        offd = [o.g[k][1 - k] for o in outer for k in range(2)]
        piece = _pack(jnp.concatenate(leaves + offd, axis=1))
        ln2_ref[rows((b * qb4 + r) // 2, xs[0].shape[0] // 2, 8), :] = piece
        return piece

    z_ref[0] = 0
    z_ref[1] = 0
    idx_ref[...] = lax.broadcasted_iota(jnp.int32, idx_ref.shape, 0)
    pc_ref[...] = jnp.zeros_like(pc_ref)
    l_ref[...] = jnp.ones_like(l_ref)
    oc_ref[...] = jnp.zeros_like(oc_ref)
    x_ref[...] = jnp.zeros_like(x_ref)

    def pin_rows(z0, t, blocks):
        n = blocks[0].shape[0]
        parts = [jnp.where(z0 == 0, t[r * n:(r + 1) * n], b) for r, b in enumerate(blocks)]
        if len(blocks) * n < t.shape[0]:
            parts.append(t[len(blocks) * n:])
        return jnp.concatenate(parts, axis=0)

    def resid(li, rws):
        if isinstance(li, int) and li == 0:
            return xio[rws, :].astype(F32)
        return jnp.where(li == 0, xio[rws, :].astype(F32), x_ref[rws, :])

    def proj(p, a0, pieces):
        z0 = z_ref[0]
        blocks = [pc[:, k * hd:(k + 1) * hd] for pc in pieces for k in range(7)]
        pins = PINS if len(pieces) < 2 else (3, 1, 4, 6, 2, 5)

        def prod(j):
            t = a0[:, j * hd:(j + 1) * hd]
            if blocks and j in pins:
                t = pin_rows(z0, t, [blocks.pop(0) for _ in range(min(2, len(blocks)))])
            return _dot(_unpack(t), _unpack(cqkv[p, j]))

        return _block(_strassen(prod))

    def next_ln(li, b, r):
        return ln1_piece(b, r, resid(li, rows(b * RB + r, T, T)), resid(li, rows(b * RB + hb + r, T, T)))

    def put_q(i, q):
        qt_ref[:, blk(i)] = _pack((q * qscale).T)

    def put_v(i, v):
        vt_ref[:, blk(i)] = _pack(v.T)

    def put_k(i, k):
        k_ref[rows(i * hb, hb, 8), :] = _pack(k)
        for t in range(RB // T):
            kv_ref[rows((i * (RB // T) + t) * 8, 8, 8), :] = _pack_pair(k[t * T:t * T + 8], k[t * T + 8:t * T + 16])

    def qkv_block(li, i):
        a0 = ln1_ref[rows(i * (hb // 2), hb // 2, 8), :]
        nxt = jnp.minimum(i + 1, nrb - 1)
        put_q(i, proj(0, a0, []))
        put_v(i, proj(2, a0, [next_ln(li, nxt, 0)]))
        put_k(i, proj(1, a0, [next_ln(li, nxt, T)]))

    def qkv_terms(p):
        grid_terms(wqkv, cqkv.at[p], 2, 0, hd, 0, hd, p * D, hd)

    x_copy(0).wait()
    x0 = xio[0:RB, :].astype(F32)
    ln1_piece(0, 0, x0[:hb], x0[hb:])
    wqkv_copy(0).wait()
    qkv_terms(0)
    q0 = proj(0, ln1_ref[0:hb // 2, :], [])
    wqkv_copy(2).wait()
    qkv_terms(2)
    put_q(0, q0)
    v0 = proj(2, ln1_ref[0:hb // 2, :], [])
    wqkv_copy(1).wait()
    x_copy(1).wait()
    qkv_terms(1)
    put_v(0, v0)
    put_k(0, proj(1, ln1_ref[0:hb // 2, :], [next_ln(0, 1, 0), next_ln(0, 1, T)]))

    def tiles_of(pc):
        return [pc[h:h + 8, k:k + T] for k in range(0, pc.shape[1], T) for h in range(0, pc.shape[0], 8)]

    def wo_phase(li):
        z0 = z_ref[0]
        side = []
        seq = {"n": 0}
        for b in range(nrb):
            ot = [[ot_ref[c * hd:(c + 1) * hd, b * RB + r * hb:b * RB + (r + 1) * hb] for c in range(2)]
                  for r in range(2)]
            terms = _lhs_terms(ot[0][0], ot[0][1], ot[1][0], ot[1][1])

            def prod(j):
                w = co[j]
                n = seq["n"] = seq["n"] + 1
                if side and n >= WOP:
                    w = jnp.concatenate(
                        [pin_rows(z0, w[:, k * T:(k + 1) * T], [side.pop(0) for _ in range(min(16, len(side)))])
                         if side else w[:, k * T:(k + 1) * T] for k in range(2)], axis=1)
                return _dot(terms[j].T.astype(BF16), _unpack(w))

            x = resid(li, blk(b)) + _block(_strassen(prod))
            xm_ref[blk(b), :] = x
            if b == 0:
                for r in range(0, qb4, RP2):
                    tl = tiles_of(ln2_piece(0, r, [x[q * qb4 + r:q * qb4 + r + RP2] for q in range(4)]))
                    side += tl + tl[-1:]
        assert not side

    def ffn_block(li, i):
        z0 = z_ref[0]
        nxt = jnp.minimum(i + 1, nrb - 1)
        a0 = ln2_ref[rows(i * (qb4 // 2), qb4 // 2, 8), :]

        def a_blk(k):
            return a0[:, k * T:(k + 1) * T]

        side = []

        for n, r in enumerate(range(0, hb // 2, RP1)):
            r = (i % 2) * (hb // 2) + r
            pc = ln1_piece(0, r, x_ref[rows(r, RP1, RP1), :], x_ref[rows(hb + r, RP1, RP1), :])
            side.append((FP1[0] + n * FP1[1], tiles_of(pc)))
        for n, r in enumerate(range(0, qb4, RP2)):
            pc = ln2_piece(nxt, r, [xm_ref[rows(nxt * RB + q * qb4 + r, RP2, RP2), :] for q in range(4)])
            side.append((FP2[0] + n * FP2[1], tiles_of(pc)))
        seq = {"n": 0}

        def pinned(w):
            n = seq["n"] = seq["n"] + 1
            for start, pc in side:
                if pc and n > start:
                    return pin_rows(z0, w, [pc.pop(0) for _ in range(min(w.shape[0] // 8, FPN, len(pc)))])
            return w

        hterms = [[] for _ in range(49)]
        mr = T // 2 // MSPLIT
        for j in range(fq):
            def part(hf_, mat):
                def inner(i1):
                    def prod(i2):
                        k = i1 * 7 + i2
                        a = a_blk(k)[hf_ * mr:(hf_ + 1) * mr]
                        w = pinned(c2gu[mat, k, :, j * T:(j + 1) * T])
                        return _dot(_unpack(a), _unpack(w))

                    return _G(_strassen(prod))

                c = _strassen(inner)
                return [c[r // 2][0].g[r % 2] + c[r // 2][1].g[r % 2] for r in range(4)]

            hs = []
            for hf_ in range(MSPLIT):
                cg, cu = part(hf_, 0), part(hf_, 1)
                hs.append([[a * b for a, b in zip(r, q)] for r, q in zip(cg, cu)])
            h = [[jnp.concatenate([hh[r][c] for hh in hs], axis=0) for c in range(4)] for r in range(4)]
            for k, t in enumerate(_terms2(_lhs_terms, h)[1]):
                hterms[k].append(t)

        def prod1(i1):
            a = _block([[a_blk(i1 * 7 + 2), a_blk(49 + 2 * i1)], [a_blk(50 + 2 * i1), a_blk(i1 * 7 + 3)]])
            w = jnp.concatenate([pinned(c1gu[0, i1]), pinned(c1gu[1, i1])], axis=1)
            return _dot(_unpack(a), _unpack(w))

        c = _strassen(prod1)
        hrem = [t.astype(BF16) for t in _lhs_terms(*[b[:, :T] * b[:, T:] for r in c for b in r])]

        def down(i1):
            rem = _dot(hrem[i1], _unpack(c1d[i1]))
            m = _strassen(lambda i2: _dot(jnp.concatenate(hterms[i1 * 7 + i2], axis=1).astype(BF16),
                                          _unpack(pinned(c2d[i1 * 7 + i2]))))
            return rem + _block(m)

        c = _strassen(down)
        assert not any(pc for _, pc in side)
        for r, q in ((1, 0), (0, 0), (0, 1), (1, 1)):
            rws, cols = rows(i * RB + r * hb, hb, hb), slice(q * hd, (q + 1) * hd)
            y = xm_ref[rws, cols] + c[r][q]
            x_ref[rws, cols] = y
            xio[rws, cols] = y.astype(xio.dtype)

            @pl.when(li == N_LAYERS - 1)
            def _():
                out_copy(i, r, q).start()

    def head_row(it, g):
        return pl.multiple_of((it % nt) * T + g * dh, dh)

    def head_rows_packed(it, g):
        return pl.ds(pl.multiple_of((it % nt) * (T // 2) + g * (dh // 2), dh // 2), dh // 2)

    def q_col(it):
        return pl.multiple_of((it // nt) * QB, QB)

    def wq(it, g):
        q = _unpack(qt_ref[head_rows_packed(it, g), pl.ds(q_col(it), QB)])
        parts = []
        if g > 0:
            parts.append(jnp.zeros((g * dh, QB), BF16))
        parts.append(q)
        if g < gph - 1:
            parts.append(jnp.zeros(((gph - 1 - g) * dh, QB), BF16))
        return jnp.concatenate(parts, axis=0)

    def q_bcast(it, g):
        qf = _unpack(qt_ref[head_rows_packed(it, g), pl.ds(q_col(it), QB)]).astype(F32)
        return [jnp.broadcast_to(qf[d:d + 1], (8, QB)) for d in range(dh)]

    def k_group(it, r16):
        return k_ref[r16 * 8:(r16 + 1) * 8, pl.ds(pl.multiple_of((it % nt) * T, T), T)]

    def pv_dot(it, g, t, pb, o):
        v = _unpack(vt_ref[head_rows_packed(it, g), t * T:(t + 1) * T])
        return o + _dot(v, pb)

    def pv_finish(it, g, l, o, write=None):
        lt = jnp.sum(l, axis=0, keepdims=True)
        res = o / lt
        dst = (pl.ds(head_row(it, g), dh), pl.ds(q_col(it), QB))
        ot_ref[dst] = res if write is None else jnp.where(write, res, ot_ref[dst])
        ok = (lt >= L_MIN) & (lt <= L_MAX)
        fin = jnp.abs(res) <= F32_MAX
        ok = fin[0:8] & fin[8:16] & ok
        return jnp.where(ok, 0.0, 1.0)

    gpt = T // 16
    ntile = gph * nc

    def ffn_weight_slice(it):
        m, k = it // 8, it % 8
        terms = grid_terms(wgu.at[m], c2gu.at[m], 4, k * 16, 16, 0, T, 0, fq * T)
        terms += grid_terms(wgu.at[m], c1gu.at[m], 2, k * 32, 32, 0, hd, fm, T)
        terms += grid_terms(wd, c2d, 4, jnp.minimum(it, fq * T // 32 - 1) * 32, 32, 0, fq * T, 0, T)
        terms += grid_terms(wd, c1d, 2, k * 16, 16, fm, T, 0, hd)
        terms += grid_terms(wo, co, 2, it * 16, 16, 0, hd, 0, hd)
        return terms

    def att_body(it, carry):
        z0 = z_ref[0]
        z1 = z_ref[1]
        prv = jnp.maximum(it - 1, 0)
        nxt = jnp.minimum(it + 1, nit - 1)
        tiles = [t[r:r + 8, n:n + T] for t in ffn_weight_slice(it)
                 for n in range(0, t.shape[1], T) for r in range(0, t.shape[0], 8)]
        per = QB // T
        tiles += [tiles[-1]] * (-len(tiles) % per)
        extra = [jnp.concatenate(tiles[k:k + per], axis=1) for k in range(0, len(tiles), per)]

        stream = [[(t, r) for r in range(gpt - 1, 0, -1)] for t in range(ntile)]
        pieces = []
        for t in range(ntile + 1):
            pc = stream[t - 1][-BOFF:] if t > 0 else []
            if t < ntile:
                pc = pc + stream[t][:-BOFF]
            pieces.append(pc)

        ws = {}
        qrows = {0: lambda d: qb_ref[d]}
        pgroups = {}
        ls = {}
        pins = []
        st = {"acc": None}
        total = nc * dh
        ngrp = (gpt - 1) * nc
        count = {}
        ocs = []

        def consume(t, r, s):
            p = jnp.exp2(s)
            g = t // nc
            p2 = p[0:8] + p[8:16]
            ls[g] = p2 if g not in ls else ls[g] + p2
            pgroups[(t, r)] = p

        def vpu_slice(g):
            step = count[g] = count.get(g, -1) + 1
            for t_ in range(step * total // ngrp, (step + 1) * total // ngrp):
                oc, d = t_ // dh, t_ % dh
                if d == 0:
                    st["k"] = kv_ref[oc * 8:(oc + 1) * 8, pl.ds(pl.multiple_of((it % nt) * T, T), T)]
                kb = jnp.take_along_axis(st["k"], idx_ref[g * dh + d], axis=1, mode="promise_in_bounds")
                kb = pltpu.bitcast(jnp.concatenate([kb, kb << 16], axis=0), F32)
                kb = jnp.concatenate([kb] * (QB // T), axis=1).reshape(2, 8, QB)
                t = kb * qrows[g](d)[None]
                st["acc"] = t if d == 0 else st["acc"] + t
                if d == dh - 1:
                    consume(g * nc + oc, 0, st["acc"].reshape(16, QB))
            if step % PSTEP == PSTEP - 1:
                return st["acc"][0]
            return pins.pop(0) if pins else None

        o = oc_ref[...]
        bad = bad_ref[...]
        for j in range(ntile + 1):
            if j < ntile and j % nc == 0:
                g = j // nc
                ws[g] = wq(it, g)
                qn = q_bcast(it, g + 1) if g < gph - 1 else q_bcast(nxt, 0)
                qrows[g + 1] = qn.__getitem__
            if j < ntile:
                pins.append(qn[j % nc])
                if j // nc == gph - 1:
                    qb_ref[j % nc] = qn[j % nc]
                for _ in range(XP if j % 8 == 0 else 1):
                    if extra:
                        pins.append(extra.pop(0))
            for g in sorted(set(t // nc for t, _ in pieces[j])):
                grp = [(t, r) for t, r in pieces[j] if t // nc == g]
                ks = [k_group(it, (t % nc) * gpt + r) for t, r in grp]
                if len(ocs) >= RUNA:
                    ks[0] = jnp.where(z1 == 0, ks[0], pltpu.bitcast(ocs[-RUNA][0:8, 0:T], U32))
                s = _dot(_unpack(jnp.concatenate(ks, axis=0)), ws[g])
                for k, (t, r) in enumerate(grp):
                    sk = s[k * 16:(k + 1) * 16]
                    pin = vpu_slice(g)
                    if pin is not None:
                        sk = pin_rows(z0, sk, [pin])
                    consume(t, r, sk)
            if j >= ntile:
                break
            t = j - 2
            if t < 0:
                o = pv_dot(prv, gph - 1, nc + t, _unpack(pc_ref[j]), o)
                if t == -1:
                    bad = jnp.maximum(bad, pv_finish(prv, gph - 1, l_ref[...], o))
            else:
                g = t // nc
                if t % nc == 0:
                    o = jnp.where(z1 == 0, 0.0, o)
                pb = jnp.concatenate([pgroups.pop((t, r)) for r in range(gpt)], axis=0)
                o = pv_dot(it, g, t % nc, pb, o)
                if t % nc == nc - 1:
                    bad = jnp.maximum(bad, pv_finish(it, g, ls[g], o))
            ocs.append(o)
        for k in range(2):
            t = ntile - 2 + k
            pc_ref[k] = _pack(jnp.concatenate([pgroups.pop((t, r)) for r in range(gpt)], axis=0))
        l_ref[...] = ls[gph - 1]
        oc_ref[...] = o
        bad_ref[...] = bad
        assert not extra and not pgroups
        return carry

    def att_tail(write):
        it = nit - 1
        o = oc_ref[...]
        for k in range(2):
            o = pv_dot(it, gph - 1, nc - 2 + k, _unpack(pc_ref[k]), o)
        bad = jnp.maximum(bad_ref[...], pv_finish(it, gph - 1, l_ref[...], o, write))
        return jnp.max(bad)

    def att_safe_body(u, carry):
        it, g = u // gph, u % gph
        tile = pl.multiple_of((it % nt) * T, T)
        cols = pl.ds(q_col(it), QB)
        qt = qt_ref[pl.ds(pl.multiple_of((it % nt) * (T // 2), T // 2), T // 2), cols]
        grp = lax.broadcasted_iota(jnp.int32, qt.shape, 0) // (dh // 2)
        w = _unpack(jnp.where(grp == g, qt, jnp.zeros_like(qt)))
        s = _dot(_unpack(k_ref[:, pl.ds(tile, T)]), w)
        p = jnp.exp2(s - jnp.max(s, axis=0, keepdims=True))
        lt = jnp.sum(p, axis=0, keepdims=True)
        o = _dot(_unpack(vt_ref[head_rows_packed(it, g), :]), p.astype(BF16))
        ot_ref[pl.ds(head_row(it, g), dh), cols] = o / lt
        return carry

    def layer(li, carry):
        def a_body(i, c):
            @pl.when(li == 0)
            def _():
                @pl.when(i + 1 < nrb)
                def _():
                    x_copy(i + 1).wait()

            qkv_block(li, i)
            return c

        lax.fori_loop(jnp.where(li == 0, 1, 0), nrb, a_body, 0)

        @pl.when(li == 0)
        def _():
            for j in range(4):
                w_copy(j).wait()

        for d, q in enumerate(q_bcast(0, 0)):
            qb_ref[d] = q
        bad_ref[...] = jnp.zeros_like(bad_ref)
        lax.fori_loop(0, nit, att_body, 0)

        def attempt(c):
            k, _ = c

            @pl.when(k == 1)
            def _():
                lax.fori_loop(0, nit * gph, att_safe_body, 0)

            unsafe = att_tail(k == 0) > 0.5
            wo_phase(li)
            return k + 1, unsafe

        lax.while_loop(lambda c: (c[0] == 0) | ((c[0] == 1) & c[1]), attempt, (0, False))

        def b_body(i, c):
            ffn_block(li, i)
            return c

        lax.fori_loop(0, nrb, b_body, 0)
        return carry

    lax.fori_loop(0, N_LAYERS, layer, 0)
    for i in range(nrb):
        for r in range(2):
            for q in range(2):
                out_copy(i, r, q).wait()


@jax.jit
def pallas_interleave_layers__softmax_full_mha__glu_gated_bilinear__prompt_kernel(
    A_x: jax.Array,
    A_wqkv: jax.Array,
    A_wo: jax.Array,
    B_x: jax.Array,
    B_w_gate: jax.Array,
    B_w_up: jax.Array,
    B_w_down: jax.Array,
):
    del B_x
    B, S, D = A_x.shape
    assert B == 1
    F = B_w_gate.shape[1]
    x2 = A_x.reshape(S, D)
    dh = D // N_HEADS
    fq = (F // T) // 4

    scratch = [
        pltpu.VMEM((S, D), A_x.dtype),
        pltpu.VMEM(A_wqkv.shape, A_wqkv.dtype),
        pltpu.VMEM(A_wo.shape, A_wo.dtype),
        pltpu.VMEM((2,) + B_w_gate.shape, B_w_gate.dtype),
        pltpu.VMEM(B_w_down.shape, B_w_down.dtype),
        pltpu.VMEM((3, 7, D // 4, D // 2), U32),
        pltpu.VMEM((7, D // 4, D // 2), U32),
        pltpu.VMEM((2, 49, T // 2, fq * T), U32),
        pltpu.VMEM((2, 7, D // 4, T), U32),
        pltpu.VMEM((49, fq * T // 2, T), U32),
        pltpu.VMEM((7, T // 2, D // 2), U32),
        pltpu.VMEM((S, D), F32),
        pltpu.VMEM((S, D), F32),
        pltpu.VMEM((S // 4, 7 * D // 2), U32),
        pltpu.VMEM((S // 8, 63 * T), U32),
        pltpu.VMEM((S // 2, D), U32),
        pltpu.VMEM((S // T * 8, D), jnp.int32),
        pltpu.VMEM((D // 2, S), U32),
        pltpu.VMEM((D // 2, S), U32),
        pltpu.VMEM((D, S), F32),
        pltpu.VMEM((2, T // 2, QB), U32),
        pltpu.VMEM((8, QB), F32),
        pltpu.VMEM((8, QB), F32),
        pltpu.VMEM((dh, QB), F32),
        pltpu.VMEM((dh, 8, QB), F32),
        pltpu.VMEM((T, 8, T), jnp.int32),
        pltpu.SMEM((2,), jnp.int32),
        pltpu.SemaphoreType.DMA((S // RB + 7,)),
    ]
    any_spec = pl.BlockSpec(memory_space=pl.ANY)
    out = pl.pallas_call(
        functools.partial(_kernel, S=S, D=D, F=F),
        out_shape=jax.ShapeDtypeStruct((S, D), A_x.dtype),
        in_specs=[any_spec] * 6,
        out_specs=any_spec,
        scratch_shapes=scratch,
        compiler_params=pltpu.CompilerParams(vmem_limit_bytes=100 * 1024 * 1024),
    )(x2, A_wqkv, A_wo, B_w_gate, B_w_up, B_w_down)
    return out.reshape(B, S, D)
```

```python
import functools
import math

import jax
import jax.numpy as jnp
from jax import lax
import jax.experimental.pallas as pl
import jax.experimental.pallas.tpu as pltpu

F32 = jnp.float32
BF16 = jnp.bfloat16
U32 = jnp.uint32

N_HEADS = 32
N_LAYERS = 2
LN_EPS = 1e-5
L_MIN, L_MAX = 2.0 ** -60, 2.0 ** 60
F32_MAX = float(jnp.finfo(jnp.float32).max)

T = 128
QB = 512
RB = 512
MSPLIT = 2
RP1 = 64
RP2 = 16

BOFF = 4
RUNA = 4
PSTEP = 2
XEND = 1
PINS = (4, 6, 2, 5)
FP1 = (592, 5)
FP2 = (604, 5)
FPN = 24
WOP = 11
WPAD = 15


def _layernorm(x):
    m = jnp.mean(x, axis=-1, keepdims=True)
    xc = x - m
    v = jnp.mean(xc * xc, axis=-1, keepdims=True)
    return xc * lax.rsqrt(v + LN_EPS)


def _pack(x):
    return pltpu.bitcast(x.astype(BF16), U32)


def _unpack(x):
    return pltpu.bitcast(x, BF16)


def _pack_pair(a, b):
    lo = pltpu.bitcast(b.astype(BF16).astype(F32), jnp.int32)
    lo = lax.shift_right_logical(lo, 16)
    bits = pltpu.bitcast(a, jnp.int32)
    mag = jnp.maximum((bits & 0x7FFFFFFF) - lo + 0x8000, 0) & 0x7FFF0000
    return (bits & jnp.int32(-2 ** 31)) | mag | lo


def _dot(a, b):
    return lax.dot_general(a, b, (((1,), (0,)), ((), ())), preferred_element_type=F32)


def _block(g):
    return jnp.concatenate([jnp.concatenate(r, axis=1) for r in g], axis=0)


class _G:
    def __init__(self, g):
        self.g = g

    def __add__(self, o):
        return _G([[a + b for a, b in zip(r, s)] for r, s in zip(self.g, o.g)])

    def __sub__(self, o):
        return _G([[a - b for a, b in zip(r, s)] for r, s in zip(self.g, o.g)])

    def flat(self):
        return self.g[0] + self.g[1]


def _lhs_terms(a11, a12, a21, a22):
    return [a11 + a22, a21 + a22, a11, a22, a11 + a12, a21 - a11, a12 - a22]


def _rhs_terms(b11, b12, b21, b22):
    return [b11 + b22, b11, b12 - b22, b21 - b11, b22, b11 + b12, b21 + b22]


def _quads(g4):
    return [_G([r[2 * c:2 * c + 2] for r in g4[2 * k:2 * k + 2]]) for k in range(2) for c in range(2)]


def _terms2(fn, g4):
    return [t for o in fn(*_quads(g4)) for t in fn(*o.flat())]


def _strassen(prod):
    m0 = prod(0)
    m3 = prod(3)
    c11 = m0 + m3
    m1 = prod(1)
    c21 = m1 + m3
    c22 = m0 - m1
    m4 = prod(4)
    c11 = c11 - m4
    c11 = c11 + prod(6)
    m2 = prod(2)
    c12 = m2 + m4
    c22 = c22 + m2
    c22 = c22 + prod(5)
    return [[c11, c12], [c21, c22]]


def _kernel(x_hbm, wqkv_hbm, wo_hbm, wg_hbm, wu_hbm, wd_hbm, out_hbm,
            xio, wqkv, wo, wgu, wd, cqkv, co, c2gu, c1gu, c2d, c1d,
            x_ref, xm_ref, ln1_ref, ln2_ref, k_ref, kv_ref, qt_ref, vt_ref, ot_ref,
            pc_ref, l_ref, bad_ref, oc_ref, qb_ref, idx_ref, z_ref, sems, *, S, D, F):
    dh = D // N_HEADS
    gph = T // dh
    nt = N_HEADS // gph
    nqb = S // QB
    nc = S // T
    nit = nt * nqb
    nrb = S // RB
    qscale = (dh ** -0.5) * math.log2(math.e)
    hb, hd = RB // 2, D // 2
    qb4 = RB // 4
    fq = (F // T) // 4
    fm = 4 * fq * T
    assert D == 4 * T and qb4 == T and F - fm == 2 * T and nrb == 4 and nit == 16

    def blk(i):
        return pl.ds(i * RB, RB) if isinstance(i, int) else pl.ds(pl.multiple_of(i * RB, RB), RB)

    def x_copy(i):
        return pltpu.make_async_copy(x_hbm.at[blk(i), :], xio.at[blk(i), :], sems.at[i])

    def out_copy(i, r, c):
        rws = pl.ds(i * RB + r * hb, hb) if isinstance(i, int) else pl.ds(pl.multiple_of(i * RB + r * hb, hb), hb)
        cols = pl.ds(c * hd, hd)
        return pltpu.make_async_copy(xio.at[rws, cols], out_hbm.at[rws, cols], sems.at[i])

    w_pairs = ((wo_hbm, wo), (wg_hbm, wgu.at[0]), (wu_hbm, wgu.at[1]), (wd_hbm, wd))

    def w_copy(j):
        return pltpu.make_async_copy(w_pairs[j][0], w_pairs[j][1], sems.at[nrb + 3 + j])

    def wqkv_copy(p):
        cols = pl.ds(p * D, D)
        return pltpu.make_async_copy(wqkv_hbm.at[:, cols], wqkv.at[:, cols], sems.at[nrb + p])

    x_copy(0).start()
    for p in (0, 2, 1):
        wqkv_copy(p).start()
    for b in range(1, nrb):
        x_copy(b).start()
    for j in (1, 2, 3, 0):
        w_copy(j).start()

    def rows(r0, n, mult):
        return pl.ds(r0, n) if isinstance(r0, int) else pl.ds(pl.multiple_of(r0, mult), n)

    def grid_terms(w, c, n, r0, nr, row0, rstep, col0, cw):
        g = [[w[rows(row0 + k * rstep + r0, nr, 16), col0 + j * cw:col0 + (j + 1) * cw].astype(F32)
              for j in range(n)] for k in range(n)]
        terms = _rhs_terms(*(g[0] + g[1])) if n == 2 else _terms2(_rhs_terms, g)
        for j, t in enumerate(terms):
            c[j, rows(r0 // 2, nr // 2, 8), :] = _pack(t)
        return terms

    def rem_terms(w, c, r0, nr):
        g = [[w[rows(k * T + r0, nr, 16), fm + j * T:fm + (j + 1) * T].astype(F32) for j in range(2)]
             for k in range(4)]
        b1, b2 = _G(g[0:2]), _G(g[2:4])
        terms = []
        for n, b in enumerate((b1 - b2, b2, b1, b2 - b1)):
            for j, t in enumerate(_rhs_terms(*b.flat())):
                c[(n // 2) * 7 + j, rows((n % 2) * (T // 2) + r0 // 2, nr // 2, 8), :] = _pack(t)
                terms.append(t)
        return terms

    def ln1_piece(b, r, xt, xb):
        lt, lb = _layernorm(xt), _layernorm(xb)
        piece = _pack(jnp.concatenate(_lhs_terms(lt[:, :hd], lt[:, hd:], lb[:, :hd], lb[:, hd:]), axis=1))
        ln1_ref[rows((b * hb + r) // 2, xt.shape[0] // 2, 8), :] = piece
        return piece

    def ln2_piece(b, r, xs):
        ls = [_layernorm(x) for x in xs]
        leaves = _terms2(_lhs_terms, [[l[:, c * T:(c + 1) * T] for c in range(4)] for l in ls])
        piece = _pack(jnp.concatenate(leaves, axis=1))
        ln2_ref[rows((b * qb4 + r) // 2, xs[0].shape[0] // 2, 8), :] = piece
        return piece

    z_ref[0] = 0
    z_ref[1] = 0
    idx_ref[...] = lax.broadcasted_iota(jnp.int32, idx_ref.shape, 0)
    pc_ref[...] = jnp.zeros_like(pc_ref)
    l_ref[...] = jnp.ones_like(l_ref)
    oc_ref[...] = jnp.zeros_like(oc_ref)
    x_ref[...] = jnp.zeros_like(x_ref)

    def pin_rows(z0, t, blocks):
        n = blocks[0].shape[0]
        parts = [jnp.where(z0 == 0, t[r * n:(r + 1) * n], b) for r, b in enumerate(blocks)]
        if len(blocks) * n < t.shape[0]:
            parts.append(t[len(blocks) * n:])
        return jnp.concatenate(parts, axis=0)

    def resid(li, rws):
        if isinstance(li, int) and li == 0:
            return xio[rws, :].astype(F32)
        return jnp.where(li == 0, xio[rws, :].astype(F32), x_ref[rws, :])

    def proj(p, a0, pieces):
        z0 = z_ref[0]
        blocks = [pc[:, k * hd:(k + 1) * hd] for pc in pieces for k in range(7)]
        pins = PINS if len(pieces) < 2 else (3, 1, 4, 6, 2, 5)

        def prod(j):
            t = a0[:, j * hd:(j + 1) * hd]
            if blocks and j in pins:
                t = pin_rows(z0, t, [blocks.pop(0) for _ in range(min(2, len(blocks)))])
            return _dot(_unpack(t), _unpack(cqkv[p, j]))

        return _block(_strassen(prod))

    def next_ln(li, b, r):
        return ln1_piece(b, r, resid(li, rows(b * RB + r, T, T)), resid(li, rows(b * RB + hb + r, T, T)))

    def put_q(i, q):
        qt_ref[:, blk(i)] = _pack((q * qscale).T)

    def put_v(i, v):
        vt_ref[:, blk(i)] = _pack(v.T)

    def put_k(i, k):
        k_ref[rows(i * hb, hb, 8), :] = _pack(k)
        for t in range(RB // T):
            kv_ref[rows((i * (RB // T) + t) * 8, 8, 8), :] = _pack_pair(k[t * T:t * T + 8], k[t * T + 8:t * T + 16])

    def qkv_block(li, i):
        a0 = ln1_ref[rows(i * (hb // 2), hb // 2, 8), :]
        nxt = jnp.minimum(i + 1, nrb - 1)
        put_q(i, proj(0, a0, []))
        put_v(i, proj(2, a0, [next_ln(li, nxt, 0)]))
        put_k(i, proj(1, a0, [next_ln(li, nxt, T)]))

    def qkv_terms(p):
        grid_terms(wqkv, cqkv.at[p], 2, 0, hd, 0, hd, p * D, hd)

    x_copy(0).wait()
    x0 = xio[0:RB, :].astype(F32)
    ln1_piece(0, 0, x0[:hb], x0[hb:])
    wqkv_copy(0).wait()
    qkv_terms(0)
    q0 = proj(0, ln1_ref[0:hb // 2, :], [])
    wqkv_copy(2).wait()
    qkv_terms(2)
    put_q(0, q0)
    v0 = proj(2, ln1_ref[0:hb // 2, :], [])
    wqkv_copy(1).wait()
    x_copy(1).wait()
    qkv_terms(1)
    put_v(0, v0)
    put_k(0, proj(1, ln1_ref[0:hb // 2, :], [next_ln(0, 1, 0), next_ln(0, 1, T)]))

    def tiles_of(pc):
        return [pc[h:h + 8, k:k + T] for k in range(0, pc.shape[1], T) for h in range(0, pc.shape[0], 8)]

    def wo_phase(li):
        z0 = z_ref[0]
        side = []
        seq = {"n": 0}
        for b in range(nrb):
            ot = [[ot_ref[c * hd:(c + 1) * hd, b * RB + r * hb:b * RB + (r + 1) * hb] for c in range(2)]
                  for r in range(2)]
            terms = _lhs_terms(ot[0][0], ot[0][1], ot[1][0], ot[1][1])

            def prod(j):
                w = co[j]
                n = seq["n"] = seq["n"] + 1
                if side and n >= WOP:
                    w = jnp.concatenate(
                        [pin_rows(z0, w[:, k * T:(k + 1) * T], [side.pop(0) for _ in range(min(16, len(side)))])
                         if side else w[:, k * T:(k + 1) * T] for k in range(2)], axis=1)
                return _dot(terms[j].T.astype(BF16), _unpack(w))

            x = resid(li, blk(b)) + _block(_strassen(prod))
            xm_ref[blk(b), :] = x
            if b == 0:
                for r in range(0, qb4, RP2):
                    tl = tiles_of(ln2_piece(0, r, [x[q * qb4 + r:q * qb4 + r + RP2] for q in range(4)]))
                    side += tl + tl[-1:] * WPAD
        assert not side

    def ffn_block(li, i):
        z0 = z_ref[0]
        nxt = jnp.minimum(i + 1, nrb - 1)
        a0 = ln2_ref[rows(i * (qb4 // 2), qb4 // 2, 8), :]

        def a_blk(k):
            return a0[:, k * T:(k + 1) * T]

        side = []

        for n, r in enumerate(range(0, hb // 2, RP1)):
            r = (i % 2) * (hb // 2) + r
            pc = ln1_piece(0, r, x_ref[rows(r, RP1, RP1), :], x_ref[rows(hb + r, RP1, RP1), :])
            side.append((FP1[0] + n * FP1[1], tiles_of(pc)))
        for n, r in enumerate(range(0, qb4, RP2)):
            pc = ln2_piece(nxt, r, [xm_ref[rows(nxt * RB + q * qb4 + r, RP2, RP2), :] for q in range(4)])
            side.append((FP2[0] + n * FP2[1], tiles_of(pc)))
        seq = {"n": 0}

        def pinned(w):
            n = seq["n"] = seq["n"] + 1
            for start, pc in side:
                if pc and n > start:
                    return pin_rows(z0, w, [pc.pop(0) for _ in range(min(w.shape[0] // 8, FPN, len(pc)))])
            return w

        hterms = [[] for _ in range(49)]
        mr = T // 2 // MSPLIT
        for j in range(fq):
            def part(hf_, mat):
                def inner(i1):
                    def prod(i2):
                        k = i1 * 7 + i2
                        a = a_blk(k)[hf_ * mr:(hf_ + 1) * mr]
                        w = pinned(c2gu[mat, k, :, j * T:(j + 1) * T])
                        return _dot(_unpack(a), _unpack(w))

                    return _G(_strassen(prod))

                c = _strassen(inner)
                return [c[r // 2][0].g[r % 2] + c[r // 2][1].g[r % 2] for r in range(4)]

            hs = []
            for hf_ in range(MSPLIT):
                cg, cu = part(hf_, 0), part(hf_, 1)
                hs.append([[a * b for a, b in zip(r, q)] for r, q in zip(cg, cu)])
            h = [[jnp.concatenate([hh[r][c] for hh in hs], axis=0) for c in range(4)] for r in range(4)]
            for k, t in enumerate(_terms2(_lhs_terms, h)):
                hterms[k].append(t)

        def rem_half(hf_):
            o1, o2 = ((2, 4), (1, 3))[hf_]

            def prod(i2):
                a = jnp.concatenate([a_blk(o1 * 7 + i2), a_blk(o2 * 7 + i2)], axis=1)
                w = jnp.concatenate([pinned(c1gu[0, hf_ * 7 + i2]), c1gu[1, hf_ * 7 + i2]], axis=1)
                return _dot(_unpack(a), _unpack(w))

            c = _strassen(prod)
            return [jnp.concatenate([c[r][q][:, :T] * c[r][q][:, T:] for r in range(2)], axis=0) for q in range(2)]

        hrem = [t.astype(BF16) for t in _lhs_terms(*(rem_half(0) + rem_half(1)))]

        def down(i1):
            rem = _dot(hrem[i1], _unpack(c1d[i1]))
            m = _strassen(lambda i2: _dot(jnp.concatenate(hterms[i1 * 7 + i2], axis=1).astype(BF16),
                                          _unpack(pinned(c2d[i1 * 7 + i2]))))
            return rem + _block(m)

        c = _strassen(down)
        assert not any(pc for _, pc in side)
        for r, q in ((1, 0), (0, 0), (0, 1), (1, 1)):
            rws, cols = rows(i * RB + r * hb, hb, hb), slice(q * hd, (q + 1) * hd)
            y = xm_ref[rws, cols] + c[r][q]
            x_ref[rws, cols] = y
            xio[rws, cols] = y.astype(xio.dtype)

            @pl.when(li == N_LAYERS - 1)
            def _():
                out_copy(i, r, q).start()

    def head_row(it, g):
        return pl.multiple_of((it % nt) * T + g * dh, dh)

    def head_rows_packed(it, g):
        return pl.ds(pl.multiple_of((it % nt) * (T // 2) + g * (dh // 2), dh // 2), dh // 2)

    def q_col(it):
        return pl.multiple_of((it // nt) * QB, QB)

    def wq(it, g):
        q = _unpack(qt_ref[head_rows_packed(it, g), pl.ds(q_col(it), QB)])
        parts = []
        if g > 0:
            parts.append(jnp.zeros((g * dh, QB), BF16))
        parts.append(q)
        if g < gph - 1:
            parts.append(jnp.zeros(((gph - 1 - g) * dh, QB), BF16))
        return jnp.concatenate(parts, axis=0)

    def q_bcast(it, g):
        qf = _unpack(qt_ref[head_rows_packed(it, g), pl.ds(q_col(it), QB)]).astype(F32)
        return [jnp.broadcast_to(qf[d:d + 1], (8, QB)) for d in range(dh)]

    def k_group(it, r16):
        return k_ref[r16 * 8:(r16 + 1) * 8, pl.ds(pl.multiple_of((it % nt) * T, T), T)]

    def pv_dot(it, g, t, pb, o):
        v = _unpack(vt_ref[head_rows_packed(it, g), t * T:(t + 1) * T])
        return o + _dot(v, pb)

    def pv_finish(it, g, l, o, write=None):
        lt = jnp.sum(l, axis=0, keepdims=True)
        res = o / lt
        dst = (pl.ds(head_row(it, g), dh), pl.ds(q_col(it), QB))
        ot_ref[dst] = res if write is None else jnp.where(write, res, ot_ref[dst])
        ok = (lt >= L_MIN) & (lt <= L_MAX)
        fin = jnp.abs(res) <= F32_MAX
        ok = fin[0:8] & fin[8:16] & ok
        return jnp.where(ok, 0.0, 1.0)

    gpt = T // 16
    ntile = gph * nc

    def ffn_weight_slice(it):
        m, k = it // 8, it % 8
        terms = grid_terms(wgu.at[m], c2gu.at[m], 4, k * 16, 16, 0, T, 0, fq * T)
        terms += rem_terms(wgu.at[m], c1gu.at[m], k * 16, 16)
        terms += grid_terms(wd, c2d, 4, jnp.minimum(it, fq * T // 32 - 1) * 32, 32, 0, fq * T, 0, T)
        terms += grid_terms(wd, c1d, 2, k * 16, 16, fm, T, 0, hd)
        terms += grid_terms(wo, co, 2, it * 16, 16, 0, hd, 0, hd)
        return terms

    def att_body(it, carry):
        z0 = z_ref[0]
        z1 = z_ref[1]
        prv = jnp.maximum(it - 1, 0)
        nxt = jnp.minimum(it + 1, nit - 1)
        tiles = [t[r:r + 8, n:n + T] for t in ffn_weight_slice(it)
                 for n in range(0, t.shape[1], T) for r in range(0, t.shape[0], 8)]
        per = QB // T
        tiles += [tiles[-1]] * (-len(tiles) % per)
        extra = [jnp.concatenate(tiles[k:k + per], axis=1) for k in range(0, len(tiles), per)]
        nextra = len(extra)

        stream = [[(t, r) for r in range(gpt - 1, 0, -1)] for t in range(ntile)]
        pieces = []
        for t in range(ntile + 1):
            pc = stream[t - 1][-BOFF:] if t > 0 else []
            if t < ntile:
                pc = pc + stream[t][:-BOFF]
            pieces.append(pc)

        ws = {}
        qrows = {0: lambda d: qb_ref[d]}
        pgroups = {}
        ls = {}
        pins = []
        st = {"acc": None}
        total = nc * dh
        ngrp = (gpt - 1) * nc
        count = {}
        ocs = []

        def consume(t, r, s):
            p = jnp.exp2(s)
            g = t // nc
            p2 = p[0:8] + p[8:16]
            ls[g] = p2 if g not in ls else ls[g] + p2
            pgroups[(t, r)] = p

        def vpu_slice(g):
            step = count[g] = count.get(g, -1) + 1
            for t_ in range(step * total // ngrp, (step + 1) * total // ngrp):
                oc, d = t_ // dh, t_ % dh
                if d == 0:
                    st["k"] = kv_ref[oc * 8:(oc + 1) * 8, pl.ds(pl.multiple_of((it % nt) * T, T), T)]
                kb = jnp.take_along_axis(st["k"], idx_ref[g * dh + d], axis=1, mode="promise_in_bounds")
                kb = pltpu.bitcast(jnp.concatenate([kb, kb << 16], axis=0), F32)
                kb = jnp.concatenate([kb] * (QB // T), axis=1).reshape(2, 8, QB)
                t = kb * qrows[g](d)[None]
                st["acc"] = t if d == 0 else st["acc"] + t
                if d == dh - 1:
                    consume(g * nc + oc, 0, st["acc"].reshape(16, QB))
            if step % PSTEP == PSTEP - 1:
                return st["acc"][0]
            return pins.pop(0) if pins else None

        o = oc_ref[...]
        bad = bad_ref[...]
        for j in range(ntile + 1):
            if j < ntile and j % nc == 0:
                g = j // nc
                ws[g] = wq(it, g)
                qn = q_bcast(it, g + 1) if g < gph - 1 else q_bcast(nxt, 0)
                qrows[g + 1] = qn.__getitem__
            if j < ntile:
                pins.append(qn[j % nc])
                if j // nc == gph - 1:
                    qb_ref[j % nc] = qn[j % nc]
                span = ntile - XEND
                for _ in range(min(j + 1, span) * nextra // span - min(j, span) * nextra // span):
                    pins.append(extra.pop(0))
            for g in sorted(set(t // nc for t, _ in pieces[j])):
                grp = [(t, r) for t, r in pieces[j] if t // nc == g]
                ks = [k_group(it, (t % nc) * gpt + r) for t, r in grp]
                if len(ocs) >= RUNA:
                    ks[0] = jnp.where(z1 == 0, ks[0], pltpu.bitcast(ocs[-RUNA][0:8, 0:T], U32))
                s = _dot(_unpack(jnp.concatenate(ks, axis=0)), ws[g])
                for k, (t, r) in enumerate(grp):
                    sk = s[k * 16:(k + 1) * 16]
                    pin = vpu_slice(g)
                    if pin is not None:
                        sk = pin_rows(z0, sk, [pin])
                    consume(t, r, sk)
            if j >= ntile:
                break
            t = j - 2
            if t < 0:
                o = pv_dot(prv, gph - 1, nc + t, _unpack(pc_ref[j]), o)
                if t == -1:
                    bad = jnp.maximum(bad, pv_finish(prv, gph - 1, l_ref[...], o))
            else:
                g = t // nc
                if t % nc == 0:
                    o = jnp.where(z1 == 0, 0.0, o)
                pb = jnp.concatenate([pgroups.pop((t, r)) for r in range(gpt)], axis=0)
                o = pv_dot(it, g, t % nc, pb, o)
                if t % nc == nc - 1:
                    bad = jnp.maximum(bad, pv_finish(it, g, ls[g], o))
            ocs.append(o)
        for k in range(2):
            t = ntile - 2 + k
            pc_ref[k] = _pack(jnp.concatenate([pgroups.pop((t, r)) for r in range(gpt)], axis=0))
        l_ref[...] = ls[gph - 1]
        oc_ref[...] = o
        bad_ref[...] = bad
        assert not extra and not pgroups
        return carry

    def att_tail(write):
        it = nit - 1
        o = oc_ref[...]
        for k in range(2):
            o = pv_dot(it, gph - 1, nc - 2 + k, _unpack(pc_ref[k]), o)
        bad = jnp.maximum(bad_ref[...], pv_finish(it, gph - 1, l_ref[...], o, write))
        return jnp.max(bad)

    def att_safe_body(u, carry):
        it, g = u // gph, u % gph
        tile = pl.multiple_of((it % nt) * T, T)
        cols = pl.ds(q_col(it), QB)
        qt = qt_ref[pl.ds(pl.multiple_of((it % nt) * (T // 2), T // 2), T // 2), cols]
        grp = lax.broadcasted_iota(jnp.int32, qt.shape, 0) // (dh // 2)
        w = _unpack(jnp.where(grp == g, qt, jnp.zeros_like(qt)))
        s = _dot(_unpack(k_ref[:, pl.ds(tile, T)]), w)
        p = jnp.exp2(s - jnp.max(s, axis=0, keepdims=True))
        lt = jnp.sum(p, axis=0, keepdims=True)
        o = _dot(_unpack(vt_ref[head_rows_packed(it, g), :]), p.astype(BF16))
        ot_ref[pl.ds(head_row(it, g), dh), cols] = o / lt
        return carry

    def layer(li, carry):
        def a_body(i, c):
            @pl.when(li == 0)
            def _():
                @pl.when(i + 1 < nrb)
                def _():
                    x_copy(i + 1).wait()

            qkv_block(li, i)
            return c

        lax.fori_loop(jnp.where(li == 0, 1, 0), nrb, a_body, 0)

        @pl.when(li == 0)
        def _():
            for j in range(4):
                w_copy(j).wait()

        for d, q in enumerate(q_bcast(0, 0)):
            qb_ref[d] = q
        bad_ref[...] = jnp.zeros_like(bad_ref)
        lax.fori_loop(0, nit, att_body, 0)

        def attempt(c):
            k, _ = c

            @pl.when(k == 1)
            def _():
                lax.fori_loop(0, nit * gph, att_safe_body, 0)

            unsafe = att_tail(k == 0) > 0.5
            wo_phase(li)
            return k + 1, unsafe

        lax.while_loop(lambda c: (c[0] == 0) | ((c[0] == 1) & c[1]), attempt, (0, False))

        def b_body(i, c):
            ffn_block(li, i)
            return c

        lax.fori_loop(0, nrb, b_body, 0)
        return carry

    lax.fori_loop(0, N_LAYERS, layer, 0)
    for i in range(nrb):
        for r in range(2):
            for q in range(2):
                out_copy(i, r, q).wait()


@jax.jit
def pallas_interleave_layers__softmax_full_mha__glu_gated_bilinear__prompt_kernel(
    A_x: jax.Array,
    A_wqkv: jax.Array,
    A_wo: jax.Array,
    B_x: jax.Array,
    B_w_gate: jax.Array,
    B_w_up: jax.Array,
    B_w_down: jax.Array,
):
    del B_x
    B, S, D = A_x.shape
    assert B == 1
    F = B_w_gate.shape[1]
    x2 = A_x.reshape(S, D)
    dh = D // N_HEADS
    fq = (F // T) // 4

    scratch = [
        pltpu.VMEM((S, D), A_x.dtype),
        pltpu.VMEM(A_wqkv.shape, A_wqkv.dtype),
        pltpu.VMEM(A_wo.shape, A_wo.dtype),
        pltpu.VMEM((2,) + B_w_gate.shape, B_w_gate.dtype),
        pltpu.VMEM(B_w_down.shape, B_w_down.dtype),
        pltpu.VMEM((3, 7, D // 4, D // 2), U32),
        pltpu.VMEM((7, D // 4, D // 2), U32),
        pltpu.VMEM((2, 49, T // 2, fq * T), U32),
        pltpu.VMEM((2, 14, T, T), U32),
        pltpu.VMEM((49, fq * T // 2, T), U32),
        pltpu.VMEM((7, T // 2, D // 2), U32),
        pltpu.VMEM((S, D), F32),
        pltpu.VMEM((S, D), F32),
        pltpu.VMEM((S // 4, 7 * D // 2), U32),
        pltpu.VMEM((S // 8, 49 * T), U32),
        pltpu.VMEM((S // 2, D), U32),
        pltpu.VMEM((S // T * 8, D), jnp.int32),
        pltpu.VMEM((D // 2, S), U32),
        pltpu.VMEM((D // 2, S), U32),
        pltpu.VMEM((D, S), F32),
        pltpu.VMEM((2, T // 2, QB), U32),
        pltpu.VMEM((8, QB), F32),
        pltpu.VMEM((8, QB), F32),
        pltpu.VMEM((dh, QB), F32),
        pltpu.VMEM((dh, 8, QB), F32),
        pltpu.VMEM((T, 8, T), jnp.int32),
        pltpu.SMEM((2,), jnp.int32),
        pltpu.SemaphoreType.DMA((S // RB + 7,)),
    ]
    any_spec = pl.BlockSpec(memory_space=pl.ANY)
    out = pl.pallas_call(
        functools.partial(_kernel, S=S, D=D, F=F),
        out_shape=jax.ShapeDtypeStruct((S, D), A_x.dtype),
        in_specs=[any_spec] * 6,
        out_specs=any_spec,
        scratch_shapes=scratch,
        compiler_params=pltpu.CompilerParams(vmem_limit_bytes=100 * 1024 * 1024),
    )(x2, A_wqkv, A_wo, B_w_gate, B_w_up, B_w_down)
    return out.reshape(B, S, D)
```

```python
import functools
import math

import jax
import jax.numpy as jnp
from jax import lax
import jax.experimental.pallas as pl
import jax.experimental.pallas.tpu as pltpu

F32 = jnp.float32
BF16 = jnp.bfloat16
U32 = jnp.uint32

N_HEADS = 32
N_LAYERS = 2
LN_EPS = 1e-5
L_MIN, L_MAX = 2.0 ** -60, 2.0 ** 60
F32_MAX = float(jnp.finfo(jnp.float32).max)

T = 128
QB = 512
RB = 512
MSPLIT = 2
RP1 = 64
RP2 = 16

VGRP = 3
HD = 24
HS = 2
BOFF = 5
RUNA = 4
PSTEP = 2
XEND = 1
PINS = (4, 6, 2, 5)
FP1 = (592, 5)
FP2 = (604, 5)
FPN = 24
WOP = 11
WPAD = 15


def _layernorm(x):
    m = jnp.mean(x, axis=-1, keepdims=True)
    xc = x - m
    v = jnp.mean(xc * xc, axis=-1, keepdims=True)
    return xc * lax.rsqrt(v + LN_EPS)


def _pack(x):
    return pltpu.bitcast(x.astype(BF16), U32)


def _unpack(x):
    return pltpu.bitcast(x, BF16)


def _pack_pair(a, b):
    lo = pltpu.bitcast(b.astype(BF16).astype(F32), jnp.int32)
    lo = lax.shift_right_logical(lo, 16)
    bits = pltpu.bitcast(a, jnp.int32)
    mag = jnp.maximum((bits & 0x7FFFFFFF) - lo + 0x8000, 0) & 0x7FFF0000
    return (bits & jnp.int32(-2 ** 31)) | mag | lo


def _dot(a, b):
    return lax.dot_general(a, b, (((1,), (0,)), ((), ())), preferred_element_type=F32)


def _block(g):
    return jnp.concatenate([jnp.concatenate(r, axis=1) for r in g], axis=0)


class _G:
    def __init__(self, g):
        self.g = g

    def __add__(self, o):
        return _G([[a + b for a, b in zip(r, s)] for r, s in zip(self.g, o.g)])

    def __sub__(self, o):
        return _G([[a - b for a, b in zip(r, s)] for r, s in zip(self.g, o.g)])

    def flat(self):
        return self.g[0] + self.g[1]


def _lhs_terms(a11, a12, a21, a22):
    return [a11 + a22, a21 + a22, a11, a22, a11 + a12, a21 - a11, a12 - a22]


def _rhs_terms(b11, b12, b21, b22):
    return [b11 + b22, b11, b12 - b22, b21 - b11, b22, b11 + b12, b21 + b22]


def _quads(g4):
    return [_G([r[2 * c:2 * c + 2] for r in g4[2 * k:2 * k + 2]]) for k in range(2) for c in range(2)]


def _terms2(fn, g4):
    return [t for o in fn(*_quads(g4)) for t in fn(*o.flat())]


def _strassen(prod):
    m0 = prod(0)
    m3 = prod(3)
    c11 = m0 + m3
    m1 = prod(1)
    c21 = m1 + m3
    c22 = m0 - m1
    m4 = prod(4)
    c11 = c11 - m4
    c11 = c11 + prod(6)
    m2 = prod(2)
    c12 = m2 + m4
    c22 = c22 + m2
    c22 = c22 + prod(5)
    return [[c11, c12], [c21, c22]]


def _kernel(x_hbm, wqkv_hbm, wo_hbm, wg_hbm, wu_hbm, wd_hbm, out_hbm,
            xio, wqkv, wo, wgu, wd, cqkv, co, c2gu, c1gu, c2d, c1d,
            x_ref, xm_ref, ln1_ref, ln2_ref, k_ref, kv_ref, qt_ref, vt_ref, ot_ref,
            pc_ref, l_ref, bad_ref, oc_ref, qb_ref, idx_ref, z_ref, sems, *, S, D, F):
    dh = D // N_HEADS
    gph = T // dh
    nt = N_HEADS // gph
    nqb = S // QB
    nc = S // T
    nit = nt * nqb
    nrb = S // RB
    qscale = (dh ** -0.5) * math.log2(math.e)
    hb, hd = RB // 2, D // 2
    qb4 = RB // 4
    fq = (F // T) // 4
    fm = 4 * fq * T
    assert D == 4 * T and qb4 == T and F - fm == 2 * T and nrb == 4 and nit == 16

    def blk(i):
        return pl.ds(i * RB, RB) if isinstance(i, int) else pl.ds(pl.multiple_of(i * RB, RB), RB)

    def x_copy(i):
        return pltpu.make_async_copy(x_hbm.at[blk(i), :], xio.at[blk(i), :], sems.at[i])

    def out_copy(i, r, c):
        rws = pl.ds(i * RB + r * hb, hb) if isinstance(i, int) else pl.ds(pl.multiple_of(i * RB + r * hb, hb), hb)
        cols = pl.ds(c * hd, hd)
        return pltpu.make_async_copy(xio.at[rws, cols], out_hbm.at[rws, cols], sems.at[i])

    w_pairs = ((wo_hbm, wo), (wg_hbm, wgu.at[0]), (wu_hbm, wgu.at[1]), (wd_hbm, wd))

    def w_copy(j):
        return pltpu.make_async_copy(w_pairs[j][0], w_pairs[j][1], sems.at[nrb + 3 + j])

    def wqkv_copy(p):
        cols = pl.ds(p * D, D)
        return pltpu.make_async_copy(wqkv_hbm.at[:, cols], wqkv.at[:, cols], sems.at[nrb + p])

    x_copy(0).start()
    wqkv_copy(0).start()
    wqkv_copy(2).start()
    x_copy(1).start()
    wqkv_copy(1).start()
    for b in range(2, nrb):
        x_copy(b).start()
    for j in (1, 2, 3, 0):
        w_copy(j).start()

    def rows(r0, n, mult):
        return pl.ds(r0, n) if isinstance(r0, int) else pl.ds(pl.multiple_of(r0, mult), n)

    def grid_terms(w, c, n, r0, nr, row0, rstep, col0, cw):
        g = [[w[rows(row0 + k * rstep + r0, nr, 16), col0 + j * cw:col0 + (j + 1) * cw].astype(F32)
              for j in range(n)] for k in range(n)]
        terms = _rhs_terms(*(g[0] + g[1])) if n == 2 else _terms2(_rhs_terms, g)
        for j, t in enumerate(terms):
            c[j, rows(r0 // 2, nr // 2, 8), :] = _pack(t)
        return terms

    def rem_terms(w, c, r0, nr):
        g = [[w[rows(k * T + r0, nr, 16), fm + j * T:fm + (j + 1) * T].astype(F32) for j in range(2)]
             for k in range(4)]
        b1, b2 = _G(g[0:2]), _G(g[2:4])
        terms = []
        for n, b in enumerate((b1 - b2, b2, b1, b2 - b1)):
            for j, t in enumerate(_rhs_terms(*b.flat())):
                c[(n // 2) * 7 + j, rows((n % 2) * (T // 2) + r0 // 2, nr // 2, 8), :] = _pack(t)
                terms.append(t)
        return terms

    def ln1_piece(b, r, xt, xb):
        lt, lb = _layernorm(xt), _layernorm(xb)
        piece = _pack(jnp.concatenate(_lhs_terms(lt[:, :hd], lt[:, hd:], lb[:, :hd], lb[:, hd:]), axis=1))
        ln1_ref[rows((b * hb + r) // 2, xt.shape[0] // 2, 8), :] = piece
        return piece

    def ln2_piece(b, r, xs):
        ls = [_layernorm(x) for x in xs]
        leaves = _terms2(_lhs_terms, [[l[:, c * T:(c + 1) * T] for c in range(4)] for l in ls])
        piece = _pack(jnp.concatenate(leaves, axis=1))
        ln2_ref[rows((b * qb4 + r) // 2, xs[0].shape[0] // 2, 8), :] = piece
        return piece

    z_ref[0] = 0
    z_ref[1] = 0
    idx_ref[...] = lax.broadcasted_iota(jnp.int32, idx_ref.shape, 0)
    pc_ref[...] = jnp.zeros_like(pc_ref)
    l_ref[...] = jnp.ones_like(l_ref)
    oc_ref[...] = jnp.zeros_like(oc_ref)
    x_ref[...] = jnp.zeros_like(x_ref)

    def pin_rows(z0, t, blocks):
        n = blocks[0].shape[0]
        parts = [jnp.where(z0 == 0, t[r * n:(r + 1) * n], b) for r, b in enumerate(blocks)]
        if len(blocks) * n < t.shape[0]:
            parts.append(t[len(blocks) * n:])
        return jnp.concatenate(parts, axis=0)

    def resid(li, rws):
        if isinstance(li, int) and li == 0:
            return xio[rws, :].astype(F32)
        return jnp.where(li == 0, xio[rws, :].astype(F32), x_ref[rws, :])

    def proj(p, a0, pieces):
        z0 = z_ref[0]
        blocks = [pc[:, k * hd:(k + 1) * hd] for pc in pieces for k in range(7)]

        def prod(j):
            t = a0[:, j * hd:(j + 1) * hd]
            if blocks and j in PINS:
                t = pin_rows(z0, t, [blocks.pop(0) for _ in range(min(2, len(blocks)))])
            return _dot(_unpack(t), _unpack(cqkv[p, j]))

        return _block(_strassen(prod))

    def next_ln(li, b, r):
        return ln1_piece(b, r, resid(li, rows(b * RB + r, T, T)), resid(li, rows(b * RB + hb + r, T, T)))

    def put_q(i, q):
        qt_ref[:, blk(i)] = _pack((q * qscale).T)

    def put_v(i, v):
        vt_ref[:, blk(i)] = _pack(v.T)

    def swap8(x):
        return jnp.concatenate([x[r + 8 - h:r + 16 - h] for r in range(0, x.shape[0], 16) for h in (0, 8)], axis=0)

    def put_k(i, k):
        k_ref[rows(i * hb, hb, 8), :] = _pack(swap8(k))
        for t in range(RB // T):
            r = t * T + VGRP * 16
            kv_ref[rows((i * (RB // T) + t) * 8, 8, 8), :] = _pack_pair(k[r:r + 8], k[r + 8:r + 16])

    def qkv_block(li, i):
        a0 = ln1_ref[rows(i * (hb // 2), hb // 2, 8), :]
        nxt = jnp.minimum(i + 1, nrb - 1)
        put_q(i, proj(0, a0, []))
        put_v(i, proj(2, a0, [next_ln(li, nxt, 0)]))
        put_k(i, proj(1, a0, [next_ln(li, nxt, T)]))

    def qkv_terms(p):
        grid_terms(wqkv, cqkv.at[p], 2, 0, hd, 0, hd, p * D, hd)

    x_copy(0).wait()
    x0 = xio[0:RB, :].astype(F32)
    ln1_piece(0, 0, x0[:hb], x0[hb:])
    wqkv_copy(0).wait()
    qkv_terms(0)
    q0 = proj(0, ln1_ref[0:hb // 2, :], [])
    wqkv_copy(2).wait()
    x_copy(1).wait()
    qkv_terms(2)
    put_q(0, q0)
    v0 = proj(2, ln1_ref[0:hb // 2, :], [next_ln(0, 1, 0)])
    wqkv_copy(1).wait()
    qkv_terms(1)
    put_v(0, v0)
    put_k(0, proj(1, ln1_ref[0:hb // 2, :], [next_ln(0, 1, T)]))

    def tiles_of(pc):
        return [pc[h:h + 8, k:k + T] for k in range(0, pc.shape[1], T) for h in range(0, pc.shape[0], 8)]

    def wo_phase(li):
        z0 = z_ref[0]
        side = []
        seq = {"n": 0}
        for b in range(nrb):
            ot = [[ot_ref[c * hd:(c + 1) * hd, b * RB + r * hb:b * RB + (r + 1) * hb] for c in range(2)]
                  for r in range(2)]
            terms = _lhs_terms(ot[0][0], ot[0][1], ot[1][0], ot[1][1])

            def prod(j):
                w = co[j]
                n = seq["n"] = seq["n"] + 1
                if side and n >= WOP:
                    w = jnp.concatenate(
                        [pin_rows(z0, w[:, k * T:(k + 1) * T], [side.pop(0) for _ in range(min(16, len(side)))])
                         if side else w[:, k * T:(k + 1) * T] for k in range(2)], axis=1)
                return _dot(terms[j].T.astype(BF16), _unpack(w))

            x = resid(li, blk(b)) + _block(_strassen(prod))
            xm_ref[blk(b), :] = x
            if b == 0:
                for r in range(0, qb4, RP2):
                    tl = tiles_of(ln2_piece(0, r, [x[q * qb4 + r:q * qb4 + r + RP2] for q in range(4)]))
                    side += tl + tl[-1:] * WPAD
        assert not side

    def ffn_block(li, i):
        z0 = z_ref[0]
        z1 = z_ref[1]
        nxt = jnp.minimum(i + 1, nrb - 1)
        a0 = ln2_ref[rows(i * (qb4 // 2), qb4 // 2, 8), :]

        def a_blk(k):
            return a0[:, k * T:(k + 1) * T]

        side = []

        for n, r in enumerate(range(0, hb // 2, RP1)):
            r = (i % 2) * (hb // 2) + r
            pc = ln1_piece(0, r, x_ref[rows(r, RP1, RP1), :], x_ref[rows(hb + r, RP1, RP1), :])
            side.append((FP1[0] + n * FP1[1], tiles_of(pc)))
        for n, r in enumerate(range(0, qb4, RP2)):
            pc = ln2_piece(nxt, r, [xm_ref[rows(nxt * RB + q * qb4 + r, RP2, RP2), :] for q in range(4)])
            side.append((FP2[0] + n * FP2[1], tiles_of(pc)))
        seq = {"n": 0}

        def pinned(w):
            n = seq["n"] = seq["n"] + 1
            for start, pc in side:
                if pc and n > start:
                    return pin_rows(z0, w, [pc.pop(0) for _ in range(min(w.shape[0] // 8, FPN, len(pc)))])
            return w

        hterms = [[[] for _ in range(MSPLIT)] for _ in range(49)]
        hq = []
        cnt = {"n": 0}

        def pin_h(a):
            cnt["n"] += 1
            if hq and cnt["n"] > HD and cnt["n"] % HS == 0:
                return pin_rows(z1, a, [hq.pop(0)])
            return a

        mr = T // 2 // MSPLIT
        for j in range(fq):
            def part(hf_, mat):
                def inner(i1):
                    def prod(i2):
                        k = i1 * 7 + i2
                        a = pin_h(a_blk(k)[hf_ * mr:(hf_ + 1) * mr])
                        w = pinned(c2gu[mat, k, :, j * T:(j + 1) * T])
                        return _dot(_unpack(a), _unpack(w))

                    return _G(_strassen(prod))

                c = _strassen(inner)
                return [c[r // 2][0].g[r % 2] + c[r // 2][1].g[r % 2] for r in range(4)]

            for hf_ in range(MSPLIT):
                cg, cu = part(hf_, 0), part(hf_, 1)
                h = [[a * b for a, b in zip(r, q)] for r, q in zip(cg, cu)]
                hq.clear()
                cnt["n"] = 0
                for k, t in enumerate(_terms2(_lhs_terms, h)):
                    hterms[k][hf_].append(_pack(t))
                    hq.append(hterms[k][hf_][-1])

        def rem_half(hf_):
            o1, o2 = ((2, 4), (1, 3))[hf_]

            def prod(i2):
                a = jnp.concatenate([a_blk(o1 * 7 + i2), a_blk(o2 * 7 + i2)], axis=1)
                w = jnp.concatenate([pinned(c1gu[0, hf_ * 7 + i2]), c1gu[1, hf_ * 7 + i2]], axis=1)
                return _dot(_unpack(a), _unpack(w))

            c = _strassen(prod)
            return [jnp.concatenate([c[r][q][:, :T] * c[r][q][:, T:] for r in range(2)], axis=0) for q in range(2)]

        hrem = [t.astype(BF16) for t in _lhs_terms(*(rem_half(0) + rem_half(1)))]

        def down(i1):
            rem = _dot(hrem[i1], _unpack(c1d[i1]))
            m = _strassen(lambda i2: _dot(_unpack(_block(hterms[i1 * 7 + i2])),
                                          _unpack(pinned(c2d[i1 * 7 + i2]))))
            return rem + _block(m)

        c = _strassen(down)
        assert not any(pc for _, pc in side)
        for r, q in ((1, 0), (0, 0), (0, 1), (1, 1)):
            rws, cols = rows(i * RB + r * hb, hb, hb), slice(q * hd, (q + 1) * hd)
            y = xm_ref[rws, cols] + c[r][q]
            x_ref[rws, cols] = y
            xio[rws, cols] = y.astype(xio.dtype)

            @pl.when(li == N_LAYERS - 1)
            def _():
                out_copy(i, r, q).start()

    def head_row(it, g):
        return pl.multiple_of((it % nt) * T + g * dh, dh)

    def head_rows_packed(it, g):
        return pl.ds(pl.multiple_of((it % nt) * (T // 2) + g * (dh // 2), dh // 2), dh // 2)

    def q_col(it):
        return pl.multiple_of((it // nt) * QB, QB)

    def wq(it, g):
        q = _unpack(qt_ref[head_rows_packed(it, g), pl.ds(q_col(it), QB)])
        parts = []
        if g > 0:
            parts.append(jnp.zeros((g * dh, QB), BF16))
        parts.append(q)
        if g < gph - 1:
            parts.append(jnp.zeros(((gph - 1 - g) * dh, QB), BF16))
        return jnp.concatenate(parts, axis=0)

    def q_bcast(it, g):
        qf = _unpack(qt_ref[head_rows_packed(it, g), pl.ds(q_col(it), QB)]).astype(F32)
        return [jnp.broadcast_to(qf[d:d + 1], (8, QB)) for d in range(dh)]

    def k_group(it, r16):
        return k_ref[r16 * 8:(r16 + 1) * 8, pl.ds(pl.multiple_of((it % nt) * T, T), T)]

    def pv_dot(it, g, t, pb, o):
        v = _unpack(vt_ref[head_rows_packed(it, g), t * T:(t + 1) * T])
        return o + _dot(v, pb)

    def pv_finish(it, g, l, o, write=None):
        lt = jnp.sum(l, axis=0, keepdims=True)
        res = o / lt
        dst = (pl.ds(head_row(it, g), dh), pl.ds(q_col(it), QB))
        ot_ref[dst] = res if write is None else jnp.where(write, res, ot_ref[dst])
        ok = (lt >= L_MIN) & (lt <= L_MAX)
        fin = jnp.abs(res) <= F32_MAX
        ok = fin[0:8] & fin[8:16] & ok
        return jnp.where(ok, 0.0, 1.0)

    gpt = T // 16
    ntile = gph * nc

    def ffn_weight_slice(it):
        m, k = it // 8, it % 8
        terms = grid_terms(wgu.at[m], c2gu.at[m], 4, k * 16, 16, 0, T, 0, fq * T)
        terms += rem_terms(wgu.at[m], c1gu.at[m], k * 16, 16)
        terms += grid_terms(wd, c2d, 4, jnp.minimum(it, fq * T // 32 - 1) * 32, 32, 0, fq * T, 0, T)
        terms += grid_terms(wd, c1d, 2, k * 16, 16, fm, T, 0, hd)
        terms += grid_terms(wo, co, 2, it * 16, 16, 0, hd, 0, hd)
        return terms

    def att_body(it, carry):
        z0 = z_ref[0]
        z1 = z_ref[1]
        prv = jnp.maximum(it - 1, 0)
        nxt = jnp.minimum(it + 1, nit - 1)
        tiles = [t[r:r + 8, n:n + T] for t in ffn_weight_slice(it)
                 for n in range(0, t.shape[1], T) for r in range(0, t.shape[0], 8)]
        per = QB // T
        tiles += [tiles[-1]] * (-len(tiles) % per)
        extra = [jnp.concatenate(tiles[k:k + per], axis=1) for k in range(0, len(tiles), per)]
        nextra = len(extra)

        stream = [[(t, r) for r in range(gpt - 1, -1, -1) if r != VGRP] for t in range(ntile)]
        work = [[] for _ in range(ntile * (gpt - 1))]
        for t in range(ntile):
            hi_ = (t + 1) * (gpt - 1) - VGRP
            lo_ = max(hi_ - (gpt - 1), 0)
            for d in range(dh):
                work[lo_ + d * (hi_ - lo_) // dh].append((t, d))
        pieces = []
        for t in range(ntile + 1):
            pc = stream[t - 1][-BOFF:] if t > 0 else []
            if t < ntile:
                pc = pc + stream[t][:-BOFF]
            pieces.append(pc)

        ws = {}
        qrows = {0: lambda d: qb_ref[d]}
        pgroups = {}
        ls = {}
        pins = []
        st = {"acc": None}
        count = {}
        ocs = []

        pend = []

        def add_l(g, p):
            ls[g] = (ls[g] + p[8:16]) + p[0:8] if g in ls else p[0:8] + p[8:16]

        def consume(t, r, s):
            p = jnp.exp2(s)
            pgroups[(t, r)] = p
            if r == VGRP:
                pend.append((t // nc, p))
                return
            add_l(t // nc, p)
            while pend:
                add_l(*pend.pop(0))

        def vpu_slice():
            step = count["n"] = count.get("n", -1) + 1
            for t_, d in work[step]:
                g, oc = t_ // nc, t_ % nc
                if d == 0:
                    st["k"] = kv_ref[oc * 8:(oc + 1) * 8, pl.ds(pl.multiple_of((it % nt) * T, T), T)]
                kb = jnp.take_along_axis(st["k"], idx_ref[g * dh + d], axis=1, mode="promise_in_bounds")
                kb = pltpu.bitcast(jnp.concatenate([kb, kb << 16], axis=0), F32)
                kb = jnp.concatenate([kb] * (QB // T), axis=1).reshape(2, 8, QB)
                t = kb * qrows[g](d)[None]
                st["acc"] = t if d == 0 else st["acc"] + t
                if d == dh - 1:
                    consume(t_, VGRP, st["acc"].reshape(16, QB))
            if step % PSTEP == PSTEP - 1:
                return st["acc"][1]
            return pins.pop(0) if pins else None

        o = oc_ref[...]
        bad = bad_ref[...]
        for j in range(ntile + 1):
            if j < ntile and j % nc == 0:
                g = j // nc
                ws[g] = wq(it, g)
                qn = q_bcast(it, g + 1) if g < gph - 1 else q_bcast(nxt, 0)
                qrows[g + 1] = qn.__getitem__
            if j < ntile:
                pins.extend(qn[0:2] if j % nc == 0 else qn[j % nc + 1:j % nc + 2])
                if j // nc == gph - 1:
                    qb_ref[j % nc] = qn[j % nc]
                span = ntile - XEND
                for _ in range(min(j + 1, span) * nextra // span - min(j, span) * nextra // span):
                    pins.append(extra.pop(0))
            for g in sorted(set(t // nc for t, _ in pieces[j])):
                grp = [(t, r) for t, r in pieces[j] if t // nc == g]
                ks = [k_group(it, (t % nc) * gpt + r) for t, r in grp]
                if len(ocs) >= RUNA:
                    ks[0] = jnp.where(z1 == 0, ks[0], pltpu.bitcast(ocs[-RUNA][0:8, 0:T], U32))
                s = _dot(_unpack(jnp.concatenate(ks, axis=0)), ws[g])
                for k, (t, r) in enumerate(grp):
                    sk = s[k * 16:(k + 1) * 16]
                    pin = vpu_slice()
                    if pin is not None:
                        sk = jnp.concatenate([sk[0:8], pin_rows(z0, sk[8:16], [pin])], axis=0)
                    consume(t, r, swap8(sk))
            if j >= ntile:
                break
            t = j - 2
            if t < 0:
                o = pv_dot(prv, gph - 1, nc + t, pc_ref[j], o)
                if t == -1:
                    bad = jnp.maximum(bad, pv_finish(prv, gph - 1, l_ref[...], o))
            else:
                g = t // nc
                if t % nc == 0:
                    o = jnp.where(z1 == 0, 0.0, o)
                pb = jnp.concatenate([pgroups.pop((t, r)) for r in range(gpt)], axis=0)
                o = pv_dot(it, g, t % nc, pb, o)
                if t % nc == nc - 1:
                    bad = jnp.maximum(bad, pv_finish(it, g, ls[g], o))
            ocs.append(o)
        for k in range(2):
            t = ntile - 2 + k
            pc_ref[k] = jnp.concatenate([pgroups.pop((t, r)) for r in range(gpt)], axis=0)
        l_ref[...] = ls[gph - 1]
        oc_ref[...] = o
        bad_ref[...] = bad
        assert not extra and not pgroups and not pend
        return carry

    def att_tail(write):
        it = nit - 1
        o = oc_ref[...]
        for k in range(2):
            o = pv_dot(it, gph - 1, nc - 2 + k, pc_ref[k], o)
        bad = jnp.maximum(bad_ref[...], pv_finish(it, gph - 1, l_ref[...], o, write))
        return jnp.max(bad)

    def att_safe_body(u, carry):
        it, g = u // gph, u % gph
        tile = pl.multiple_of((it % nt) * T, T)
        cols = pl.ds(q_col(it), QB)
        qt = qt_ref[pl.ds(pl.multiple_of((it % nt) * (T // 2), T // 2), T // 2), cols]
        grp = lax.broadcasted_iota(jnp.int32, qt.shape, 0) // (dh // 2)
        w = _unpack(jnp.where(grp == g, qt, jnp.zeros_like(qt)))
        s = _dot(_unpack(k_ref[:, pl.ds(tile, T)]), w)
        s = swap8(s)
        p = jnp.exp2(s - jnp.max(s, axis=0, keepdims=True))
        lt = jnp.sum(p, axis=0, keepdims=True)
        o = _dot(_unpack(vt_ref[head_rows_packed(it, g), :]), p.astype(BF16))
        ot_ref[pl.ds(head_row(it, g), dh), cols] = o / lt
        return carry

    def layer(li, carry):
        def a_body(i, c):
            @pl.when(li == 0)
            def _():
                @pl.when(i + 1 < nrb)
                def _():
                    x_copy(i + 1).wait()

            qkv_block(li, i)
            return c

        lax.fori_loop(jnp.where(li == 0, 1, 0), nrb, a_body, 0)

        @pl.when(li == 0)
        def _():
            for j in range(4):
                w_copy(j).wait()

        for d, q in enumerate(q_bcast(0, 0)):
            qb_ref[d] = q
        bad_ref[...] = jnp.zeros_like(bad_ref)
        lax.fori_loop(0, nit, att_body, 0)

        def attempt(c):
            k, _ = c

            @pl.when(k == 1)
            def _():
                lax.fori_loop(0, nit * gph, att_safe_body, 0)

            unsafe = att_tail(k == 0) > 0.5
            wo_phase(li)
            return k + 1, unsafe

        lax.while_loop(lambda c: (c[0] == 0) | ((c[0] == 1) & c[1]), attempt, (0, False))

        def b_body(i, c):
            ffn_block(li, i)
            return c

        lax.fori_loop(0, nrb, b_body, 0)
        return carry

    lax.fori_loop(0, N_LAYERS, layer, 0)
    for i in range(nrb):
        for r in range(2):
            for q in range(2):
                out_copy(i, r, q).wait()


@jax.jit
def pallas_interleave_layers__softmax_full_mha__glu_gated_bilinear__prompt_kernel(
    A_x: jax.Array,
    A_wqkv: jax.Array,
    A_wo: jax.Array,
    B_x: jax.Array,
    B_w_gate: jax.Array,
    B_w_up: jax.Array,
    B_w_down: jax.Array,
):
    del B_x
    B, S, D = A_x.shape
    assert B == 1
    F = B_w_gate.shape[1]
    x2 = A_x.reshape(S, D)
    dh = D // N_HEADS
    fq = (F // T) // 4

    scratch = [
        pltpu.VMEM((S, D), A_x.dtype),
        pltpu.VMEM(A_wqkv.shape, A_wqkv.dtype),
        pltpu.VMEM(A_wo.shape, A_wo.dtype),
        pltpu.VMEM((2,) + B_w_gate.shape, B_w_gate.dtype),
        pltpu.VMEM(B_w_down.shape, B_w_down.dtype),
        pltpu.VMEM((3, 7, D // 4, D // 2), U32),
        pltpu.VMEM((7, D // 4, D // 2), U32),
        pltpu.VMEM((2, 49, T // 2, fq * T), U32),
        pltpu.VMEM((2, 14, T, T), U32),
        pltpu.VMEM((49, fq * T // 2, T), U32),
        pltpu.VMEM((7, T // 2, D // 2), U32),
        pltpu.VMEM((S, D), F32),
        pltpu.VMEM((S, D), F32),
        pltpu.VMEM((S // 4, 7 * D // 2), U32),
        pltpu.VMEM((S // 8, 49 * T), U32),
        pltpu.VMEM((S // 2, D), U32),
        pltpu.VMEM((S // T * 8, D), jnp.int32),
        pltpu.VMEM((D // 2, S), U32),
        pltpu.VMEM((D // 2, S), U32),
        pltpu.VMEM((D, S), F32),
        pltpu.VMEM((2, T, QB), F32),
        pltpu.VMEM((8, QB), F32),
        pltpu.VMEM((8, QB), F32),
        pltpu.VMEM((dh, QB), F32),
        pltpu.VMEM((dh, 8, QB), F32),
        pltpu.VMEM((T, 8, T), jnp.int32),
        pltpu.SMEM((2,), jnp.int32),
        pltpu.SemaphoreType.DMA((S // RB + 7,)),
    ]
    any_spec = pl.BlockSpec(memory_space=pl.ANY)
    out = pl.pallas_call(
        functools.partial(_kernel, S=S, D=D, F=F),
        out_shape=jax.ShapeDtypeStruct((S, D), A_x.dtype),
        in_specs=[any_spec] * 6,
        out_specs=any_spec,
        scratch_shapes=scratch,
        compiler_params=pltpu.CompilerParams(vmem_limit_bytes=100 * 1024 * 1024),
    )(x2, A_wqkv, A_wo, B_w_gate, B_w_up, B_w_down)
    return out.reshape(B, S, D)
```

```python
import functools
import math

import jax
import jax.numpy as jnp
from jax import lax
import jax.experimental.pallas as pl
import jax.experimental.pallas.tpu as pltpu

F32 = jnp.float32
BF16 = jnp.bfloat16
U32 = jnp.uint32

N_HEADS = 32
N_LAYERS = 2
LN_EPS = 1e-5
L_MIN, L_MAX = 2.0 ** -60, 2.0 ** 60
F32_MAX = float(jnp.finfo(jnp.float32).max)

T = 128
QB = 512
RB = 512
MSPLIT = 2
RP1 = 64
RP2 = 16

VGRP = 3
HD = 24
HS = 2
BOFF = 5
RUNA = 4
PSTEP = 2
XEND = 1
PINS = (4, 6, 2, 5)
FP1 = (592, 5)
FP2 = (604, 5)
FPN = 24
WOP = 10
WPN = 11


def _layernorm(x):
    m = jnp.mean(x, axis=-1, keepdims=True)
    xc = x - m
    v = jnp.mean(xc * xc, axis=-1, keepdims=True)
    return xc * lax.rsqrt(v + LN_EPS)


def _pack(x):
    return pltpu.bitcast(x.astype(BF16), U32)


def _unpack(x):
    return pltpu.bitcast(x, BF16)


def _pack_pair(a, b):
    lo = pltpu.bitcast(b.astype(BF16).astype(F32), jnp.int32)
    lo = lax.shift_right_logical(lo, 16)
    bits = pltpu.bitcast(a, jnp.int32)
    mag = jnp.maximum((bits & 0x7FFFFFFF) - lo + 0x8000, 0) & 0x7FFF0000
    return (bits & jnp.int32(-2 ** 31)) | mag | lo


def _dot(a, b):
    return lax.dot_general(a, b, (((1,), (0,)), ((), ())), preferred_element_type=F32)


def _block(g):
    return jnp.concatenate([jnp.concatenate(r, axis=1) for r in g], axis=0)


class _G:
    def __init__(self, g):
        self.g = g

    def __add__(self, o):
        return _G([[a + b for a, b in zip(r, s)] for r, s in zip(self.g, o.g)])

    def __sub__(self, o):
        return _G([[a - b for a, b in zip(r, s)] for r, s in zip(self.g, o.g)])

    def flat(self):
        return self.g[0] + self.g[1]


def _lhs_terms(a11, a12, a21, a22):
    return [a11 + a22, a21 + a22, a11, a22, a11 + a12, a21 - a11, a12 - a22]


def _rhs_terms(b11, b12, b21, b22):
    return [b11 + b22, b11, b12 - b22, b21 - b11, b22, b11 + b12, b21 + b22]


def _quads(g4):
    return [_G([r[2 * c:2 * c + 2] for r in g4[2 * k:2 * k + 2]]) for k in range(2) for c in range(2)]


def _terms2(fn, g4):
    return [t for o in fn(*_quads(g4)) for t in fn(*o.flat())]


def _strassen(prod):
    m0 = prod(0)
    m3 = prod(3)
    c11 = m0 + m3
    m1 = prod(1)
    c21 = m1 + m3
    c22 = m0 - m1
    m4 = prod(4)
    c11 = c11 - m4
    c11 = c11 + prod(6)
    m2 = prod(2)
    c12 = m2 + m4
    c22 = c22 + m2
    c22 = c22 + prod(5)
    return [[c11, c12], [c21, c22]]


def _kernel(x_hbm, wqkv_hbm, wo_hbm, wg_hbm, wu_hbm, wd_hbm, out_hbm,
            xio, wqkv, wo, wgu, wd, cqkv, co, c2gu, c1gu, c2d, c1d,
            x_ref, xm_ref, ln1_ref, ln2_ref, k_ref, kv_ref, qt_ref, vt_ref, ot_ref,
            pc_ref, l_ref, bad_ref, oc_ref, qb_ref, idx_ref, z_ref, sems, *, S, D, F):
    dh = D // N_HEADS
    gph = T // dh
    nt = N_HEADS // gph
    nqb = S // QB
    nc = S // T
    nit = nt * nqb
    nrb = S // RB
    qscale = (dh ** -0.5) * math.log2(math.e)
    hb, hd = RB // 2, D // 2
    qb4 = RB // 4
    fq = (F // T) // 4
    fm = 4 * fq * T
    assert D == 4 * T and qb4 == T and F - fm == 2 * T and nrb == 4 and nit == 16

    def blk(i):
        return pl.ds(i * RB, RB) if isinstance(i, int) else pl.ds(pl.multiple_of(i * RB, RB), RB)

    def x_copy(i):
        return pltpu.make_async_copy(x_hbm.at[blk(i), :], xio.at[blk(i), :], sems.at[i])

    def out_copy(i, r, c):
        rws = pl.ds(i * RB + r * hb, hb) if isinstance(i, int) else pl.ds(pl.multiple_of(i * RB + r * hb, hb), hb)
        cols = pl.ds(c * hd, hd)
        return pltpu.make_async_copy(xio.at[rws, cols], out_hbm.at[rws, cols], sems.at[i])

    w_pairs = ((wo_hbm, wo), (wg_hbm, wgu.at[0]), (wu_hbm, wgu.at[1]), (wd_hbm, wd))

    def w_copy(j):
        return pltpu.make_async_copy(w_pairs[j][0], w_pairs[j][1], sems.at[nrb + 3 + j])

    def wqkv_copy(p):
        cols = pl.ds(p * D, D)
        return pltpu.make_async_copy(wqkv_hbm.at[:, cols], wqkv.at[:, cols], sems.at[nrb + p])

    x_copy(0).start()
    wqkv_copy(0).start()
    wqkv_copy(2).start()
    x_copy(1).start()
    wqkv_copy(1).start()
    for b in range(2, nrb):
        x_copy(b).start()
    for j in (1, 2, 3, 0):
        w_copy(j).start()

    def rows(r0, n, mult):
        return pl.ds(r0, n) if isinstance(r0, int) else pl.ds(pl.multiple_of(r0, mult), n)

    def grid_terms(w, c, n, r0, nr, row0, rstep, col0, cw):
        g = [[w[rows(row0 + k * rstep + r0, nr, 16), col0 + j * cw:col0 + (j + 1) * cw].astype(F32)
              for j in range(n)] for k in range(n)]
        terms = _rhs_terms(*(g[0] + g[1])) if n == 2 else _terms2(_rhs_terms, g)
        for j, t in enumerate(terms):
            c[j, rows(r0 // 2, nr // 2, 8), :] = _pack(t)
        return terms

    def rem_terms(w, c, r0, nr):
        g = [[w[rows(k * T + r0, nr, 16), fm + j * T:fm + (j + 1) * T].astype(F32) for j in range(2)]
             for k in range(4)]
        b1, b2 = _G(g[0:2]), _G(g[2:4])
        terms = []
        for n, b in enumerate((b1 - b2, b2, b1, b2 - b1)):
            for j, t in enumerate(_rhs_terms(*b.flat())):
                c[(n // 2) * 7 + j, rows((n % 2) * (T // 2) + r0 // 2, nr // 2, 8), :] = _pack(t)
                terms.append(t)
        return terms

    def ln1_piece(b, r, xt, xb):
        lt, lb = _layernorm(xt), _layernorm(xb)
        piece = _pack(jnp.concatenate(_lhs_terms(lt[:, :hd], lt[:, hd:], lb[:, :hd], lb[:, hd:]), axis=1))
        ln1_ref[rows((b * hb + r) // 2, xt.shape[0] // 2, 8), :] = piece
        return piece

    def ln2_piece(b, r, xs):
        ls = [_layernorm(x) for x in xs]
        leaves = _terms2(_lhs_terms, [[l[:, c * T:(c + 1) * T] for c in range(4)] for l in ls])
        piece = _pack(jnp.concatenate(leaves, axis=1))
        ln2_ref[rows((b * qb4 + r) // 2, xs[0].shape[0] // 2, 8), :] = piece
        return piece

    z_ref[0] = 0
    z_ref[1] = 0
    idx_ref[...] = lax.broadcasted_iota(jnp.int32, idx_ref.shape, 0)
    pc_ref[...] = jnp.zeros_like(pc_ref)
    l_ref[...] = jnp.ones_like(l_ref)
    oc_ref[...] = jnp.zeros_like(oc_ref)
    x_ref[...] = jnp.zeros_like(x_ref)
    ot_ref[D - dh:, S - QB:] = jnp.zeros((dh, QB), F32)

    def pin_rows(z0, t, blocks):
        n = blocks[0].shape[0]
        parts = [jnp.where(z0 == 0, t[r * n:(r + 1) * n], b) for r, b in enumerate(blocks)]
        if len(blocks) * n < t.shape[0]:
            parts.append(t[len(blocks) * n:])
        return jnp.concatenate(parts, axis=0)

    def resid(li, rws):
        if isinstance(li, int) and li == 0:
            return xio[rws, :].astype(F32)
        return jnp.where(li == 0, xio[rws, :].astype(F32), x_ref[rws, :])

    def proj(p, a0, pieces):
        z0 = z_ref[0]
        blocks = [pc[:, k * hd:(k + 1) * hd] for pc in pieces for k in range(7)]

        def prod(j):
            t = a0[:, j * hd:(j + 1) * hd]
            if blocks and j in PINS:
                t = pin_rows(z0, t, [blocks.pop(0) for _ in range(min(2, len(blocks)))])
            return _dot(_unpack(t), _unpack(cqkv[p, j]))

        return _block(_strassen(prod))

    def next_ln(li, b, r):
        return ln1_piece(b, r, resid(li, rows(b * RB + r, T, T)), resid(li, rows(b * RB + hb + r, T, T)))

    def put_q(i, q):
        qt_ref[:, blk(i)] = _pack((q * qscale).T)

    def put_v(i, v):
        vt_ref[:, blk(i)] = _pack(v.T)

    def swap8(x):
        return jnp.concatenate([x[r + 8 - h:r + 16 - h] for r in range(0, x.shape[0], 16) for h in (0, 8)], axis=0)

    def put_k(i, k):
        k_ref[rows(i * hb, hb, 8), :] = _pack(swap8(k))
        for t in range(RB // T):
            r = t * T + VGRP * 16
            kv_ref[rows((i * (RB // T) + t) * 8, 8, 8), :] = _pack_pair(k[r:r + 8], k[r + 8:r + 16])

    def qkv_block(li, i):
        a0 = ln1_ref[rows(i * (hb // 2), hb // 2, 8), :]
        nxt = jnp.minimum(i + 1, nrb - 1)
        put_q(i, proj(0, a0, []))
        put_v(i, proj(2, a0, [next_ln(li, nxt, 0)]))
        put_k(i, proj(1, a0, [next_ln(li, nxt, T)]))

    def qkv_terms(p):
        grid_terms(wqkv, cqkv.at[p], 2, 0, hd, 0, hd, p * D, hd)

    x_copy(0).wait()
    x0 = xio[0:RB, :].astype(F32)
    ln1_piece(0, 0, x0[:hb], x0[hb:])
    wqkv_copy(0).wait()
    qkv_terms(0)
    q0 = proj(0, ln1_ref[0:hb // 2, :], [])
    wqkv_copy(2).wait()
    x_copy(1).wait()
    qkv_terms(2)
    put_q(0, q0)
    v0 = proj(2, ln1_ref[0:hb // 2, :], [next_ln(0, 1, 0)])
    wqkv_copy(1).wait()
    qkv_terms(1)
    put_v(0, v0)
    put_k(0, proj(1, ln1_ref[0:hb // 2, :], [next_ln(0, 1, T)]))

    def tiles_of(pc):
        return [pc[h:h + 8, k:k + T] for k in range(0, pc.shape[1], T) for h in range(0, pc.shape[0], 8)]

    def wo_phase(li):
        z0 = z_ref[0]
        side = []
        seq = {"n": 0}
        for b in range(nrb):
            ot = [[ot_ref[c * hd:(c + 1) * hd, b * RB + r * hb:b * RB + (r + 1) * hb] for c in range(2)]
                  for r in range(2)]
            terms = _lhs_terms(ot[0][0], ot[0][1], ot[1][0], ot[1][1])

            def prod(j):
                w = co[j]
                n = seq["n"] = seq["n"] + 1
                if side and n >= WOP:
                    w = jnp.concatenate(
                        [pin_rows(z0, w[:, k * T:(k + 1) * T], [side.pop(0) for _ in range(min(WPN, len(side)))])
                         if side else w[:, k * T:(k + 1) * T] for k in range(2)], axis=1)
                return _dot(terms[j].T.astype(BF16), _unpack(w))

            x = resid(li, blk(b)) + _block(_strassen(prod))
            xm_ref[blk(b), :] = x
            if b == 0:
                for r in range(0, qb4, RP2):
                    side += tiles_of(ln2_piece(0, r, [x[q * qb4 + r:q * qb4 + r + RP2] for q in range(4)]))
        assert not side

    def ffn_block(li, i):
        z0 = z_ref[0]
        z1 = z_ref[1]
        nxt = jnp.minimum(i + 1, nrb - 1)
        a0 = ln2_ref[rows(i * (qb4 // 2), qb4 // 2, 8), :]

        def a_blk(k):
            return a0[:, k * T:(k + 1) * T]

        side = []

        for n, r in enumerate(range(0, hb // 2, RP1)):
            r = (i % 2) * (hb // 2) + r
            pc = ln1_piece(0, r, x_ref[rows(r, RP1, RP1), :], x_ref[rows(hb + r, RP1, RP1), :])
            side.append((FP1[0] + n * FP1[1], tiles_of(pc)))
        for n, r in enumerate(range(0, qb4, RP2)):
            pc = ln2_piece(nxt, r, [xm_ref[rows(nxt * RB + q * qb4 + r, RP2, RP2), :] for q in range(4)])
            side.append((FP2[0] + n * FP2[1], tiles_of(pc)))
        seq = {"n": 0}

        def pinned(w):
            n = seq["n"] = seq["n"] + 1
            for start, pc in side:
                if pc and n > start:
                    return pin_rows(z0, w, [pc.pop(0) for _ in range(min(w.shape[0] // 8, FPN, len(pc)))])
            return w

        hterms = [[[] for _ in range(MSPLIT)] for _ in range(49)]
        hq = []
        cnt = {"n": 0}

        def pin_h(a):
            cnt["n"] += 1
            if hq and cnt["n"] > HD and cnt["n"] % HS == 0:
                return pin_rows(z1, a, [hq.pop(0)])
            return a

        mr = T // 2 // MSPLIT
        for j in range(fq):
            def part(hf_, mat):
                def inner(i1):
                    def prod(i2):
                        k = i1 * 7 + i2
                        a = pin_h(a_blk(k)[hf_ * mr:(hf_ + 1) * mr])
                        w = pinned(c2gu[mat, k, :, j * T:(j + 1) * T])
                        return _dot(_unpack(a), _unpack(w))

                    return _G(_strassen(prod))

                c = _strassen(inner)
                return [c[r // 2][0].g[r % 2] + c[r // 2][1].g[r % 2] for r in range(4)]

            for hf_ in range(MSPLIT):
                cg, cu = part(hf_, 0), part(hf_, 1)
                h = [[a * b for a, b in zip(r, q)] for r, q in zip(cg, cu)]
                hq.clear()
                cnt["n"] = 0
                for k, t in enumerate(_terms2(_lhs_terms, h)):
                    hterms[k][hf_].append(_pack(t))
                    hq.append(hterms[k][hf_][-1])

        def rem_half(hf_):
            o1, o2 = ((2, 4), (1, 3))[hf_]

            def prod(i2):
                a = jnp.concatenate([a_blk(o1 * 7 + i2), a_blk(o2 * 7 + i2)], axis=1)
                w = jnp.concatenate([pinned(c1gu[0, hf_ * 7 + i2]), c1gu[1, hf_ * 7 + i2]], axis=1)
                return _dot(_unpack(a), _unpack(w))

            c = _strassen(prod)
            return [jnp.concatenate([c[r][q][:, :T] * c[r][q][:, T:] for r in range(2)], axis=0) for q in range(2)]

        hrem = [t.astype(BF16) for t in _lhs_terms(*(rem_half(0) + rem_half(1)))]

        def down(i1):
            rem = _dot(hrem[i1], _unpack(c1d[i1]))
            m = _strassen(lambda i2: _dot(_unpack(_block(hterms[i1 * 7 + i2])),
                                          _unpack(pinned(c2d[i1 * 7 + i2]))))
            return rem + _block(m)

        c = _strassen(down)
        assert not any(pc for _, pc in side)
        for r, q in ((1, 0), (0, 0), (0, 1), (1, 1)):
            rws, cols = rows(i * RB + r * hb, hb, hb), slice(q * hd, (q + 1) * hd)
            y = xm_ref[rws, cols] + c[r][q]
            x_ref[rws, cols] = y
            xio[rws, cols] = y.astype(xio.dtype)

            @pl.when(li == N_LAYERS - 1)
            def _():
                out_copy(i, r, q).start()

    def head_row(it, g):
        return pl.multiple_of((it % nt) * T + g * dh, dh)

    def head_rows_packed(it, g):
        return pl.ds(pl.multiple_of((it % nt) * (T // 2) + g * (dh // 2), dh // 2), dh // 2)

    def q_col(it):
        return pl.multiple_of((it // nt) * QB, QB)

    def wq(it, g):
        q = _unpack(qt_ref[head_rows_packed(it, g), pl.ds(q_col(it), QB)])
        parts = []
        if g > 0:
            parts.append(jnp.zeros((g * dh, QB), BF16))
        parts.append(q)
        if g < gph - 1:
            parts.append(jnp.zeros(((gph - 1 - g) * dh, QB), BF16))
        return jnp.concatenate(parts, axis=0)

    def q_bcast(it, g):
        qf = _unpack(qt_ref[head_rows_packed(it, g), pl.ds(q_col(it), QB)]).astype(F32)
        return [jnp.broadcast_to(qf[d:d + 1], (8, QB)) for d in range(dh)]

    def k_group(it, r16):
        return k_ref[r16 * 8:(r16 + 1) * 8, pl.ds(pl.multiple_of((it % nt) * T, T), T)]

    def pv_dot(it, g, t, pb, o):
        v = _unpack(vt_ref[head_rows_packed(it, g), t * T:(t + 1) * T])
        return o + _dot(v, pb)

    def pv_finish(it, g, l, o, write=None):
        lt = jnp.sum(l, axis=0, keepdims=True)
        res = o / lt
        dst = (pl.ds(head_row(it, g), dh), pl.ds(q_col(it), QB))
        ot_ref[dst] = res if write is None else jnp.where(write, res, ot_ref[dst])
        ok = (lt >= L_MIN) & (lt <= L_MAX)
        fin = jnp.abs(res) <= F32_MAX
        ok = fin[0:8] & fin[8:16] & ok
        return jnp.where(ok, 0.0, 1.0)

    gpt = T // 16
    ntile = gph * nc

    def ffn_weight_slice(it):
        m, k = it // 8, it % 8
        terms = grid_terms(wgu.at[m], c2gu.at[m], 4, k * 16, 16, 0, T, 0, fq * T)
        terms += rem_terms(wgu.at[m], c1gu.at[m], k * 16, 16)
        terms += grid_terms(wd, c2d, 4, jnp.minimum(it, fq * T // 32 - 1) * 32, 32, 0, fq * T, 0, T)
        terms += grid_terms(wd, c1d, 2, k * 16, 16, fm, T, 0, hd)
        terms += grid_terms(wo, co, 2, it * 16, 16, 0, hd, 0, hd)
        return terms

    def att_body(it, carry):
        z0 = z_ref[0]
        z1 = z_ref[1]
        prv = jnp.maximum(it - 1, 0)
        nxt = jnp.minimum(it + 1, nit - 1)
        tiles = [t[r:r + 8, n:n + T] for t in ffn_weight_slice(it)
                 for n in range(0, t.shape[1], T) for r in range(0, t.shape[0], 8)]
        per = QB // T
        tiles += [tiles[-1]] * (-len(tiles) % per)
        extra = [jnp.concatenate(tiles[k:k + per], axis=1) for k in range(0, len(tiles), per)]
        nextra = len(extra)

        stream = [[(t, r) for r in range(gpt - 1, -1, -1) if r != VGRP] for t in range(ntile)]
        work = [[] for _ in range(ntile * (gpt - 1))]
        for t in range(ntile):
            hi_ = (t + 1) * (gpt - 1) - VGRP
            lo_ = max(hi_ - (gpt - 1), 0)
            for d in range(dh):
                work[lo_ + d * (hi_ - lo_) // dh].append((t, d))
        pieces = []
        for t in range(ntile + 1):
            pc = stream[t - 1][-BOFF:] if t > 0 else []
            if t < ntile:
                pc = pc + stream[t][:-BOFF]
            pieces.append(pc)

        ws = {}
        qrows = {0: lambda d: qb_ref[d]}
        pgroups = {}
        ls = {}
        pins = []
        st = {"acc": None}
        count = {}
        ocs = []

        pend = []

        def add_l(g, p):
            ls[g] = (ls[g] + p[8:16]) + p[0:8] if g in ls else p[0:8] + p[8:16]

        def consume(t, r, s):
            p = jnp.exp2(s)
            pgroups[(t, r)] = p
            if r == VGRP:
                pend.append((t // nc, p))
                return
            add_l(t // nc, p)
            while pend:
                add_l(*pend.pop(0))

        def vpu_slice():
            step = count["n"] = count.get("n", -1) + 1
            for t_, d in work[step]:
                g, oc = t_ // nc, t_ % nc
                if d == 0:
                    st["k"] = kv_ref[oc * 8:(oc + 1) * 8, pl.ds(pl.multiple_of((it % nt) * T, T), T)]
                kb = jnp.take_along_axis(st["k"], idx_ref[g * dh + d], axis=1, mode="promise_in_bounds")
                kb = pltpu.bitcast(jnp.concatenate([kb, kb << 16], axis=0), F32)
                kb = jnp.concatenate([kb] * (QB // T), axis=1).reshape(2, 8, QB)
                t = kb * qrows[g](d)[None]
                st["acc"] = t if d == 0 else st["acc"] + t
                if d == dh - 1:
                    consume(t_, VGRP, st["acc"].reshape(16, QB))
            if step % PSTEP == PSTEP - 1:
                return st["acc"][1]
            return pins.pop(0) if pins else None

        o = oc_ref[...]
        bad = bad_ref[...]
        for j in range(ntile + 1):
            if j < ntile and j % nc == 0:
                g = j // nc
                ws[g] = wq(it, g)
                qn = q_bcast(it, g + 1) if g < gph - 1 else q_bcast(nxt, 0)
                qrows[g + 1] = qn.__getitem__
            if j < ntile:
                pins.extend(qn[0:2] if j % nc == 0 else qn[j % nc + 1:j % nc + 2])
                if j // nc == gph - 1:
                    qb_ref[j % nc] = qn[j % nc]
                span = ntile - XEND
                for _ in range(min(j + 1, span) * nextra // span - min(j, span) * nextra // span):
                    pins.append(extra.pop(0))
            for g in sorted(set(t // nc for t, _ in pieces[j])):
                grp = [(t, r) for t, r in pieces[j] if t // nc == g]
                ks = [k_group(it, (t % nc) * gpt + r) for t, r in grp]
                if len(ocs) >= RUNA:
                    ks[0] = jnp.where(z1 == 0, ks[0], pltpu.bitcast(ocs[-RUNA][0:8, 0:T], U32))
                s = _dot(_unpack(jnp.concatenate(ks, axis=0)), ws[g])
                for k, (t, r) in enumerate(grp):
                    sk = s[k * 16:(k + 1) * 16]
                    pin = vpu_slice()
                    if pin is not None:
                        sk = jnp.concatenate([sk[0:8], pin_rows(z0, sk[8:16], [pin])], axis=0)
                    consume(t, r, swap8(sk))
            if j >= ntile:
                break
            t = j - 2
            if t < 0:
                o = pv_dot(prv, gph - 1, nc + t, pc_ref[j], o)
                if t == -1:
                    bad = jnp.maximum(bad, pv_finish(prv, gph - 1, l_ref[...], o))
            else:
                g = t // nc
                if t % nc == 0:
                    o = jnp.where(z1 == 0, 0.0, o)
                pb = jnp.concatenate([pgroups.pop((t, r)) for r in range(gpt)], axis=0)
                o = pv_dot(it, g, t % nc, pb, o)
                if t % nc == nc - 1:
                    bad = jnp.maximum(bad, pv_finish(it, g, ls[g], o))
            ocs.append(o)
        for k in range(2):
            t = ntile - 2 + k
            pc_ref[k] = jnp.concatenate([pgroups.pop((t, r)) for r in range(gpt)], axis=0)
        l_ref[...] = ls[gph - 1]
        oc_ref[...] = o
        bad_ref[...] = bad
        assert not extra and not pgroups and not pend
        return carry

    def att_tail(write):
        it = nit - 1
        o = oc_ref[...]
        for k in range(2):
            o = pv_dot(it, gph - 1, nc - 2 + k, pc_ref[k], o)
        bad = jnp.maximum(bad_ref[...], pv_finish(it, gph - 1, l_ref[...], o, write))
        return jnp.max(bad)

    def att_safe_body(u, carry):
        it, g = u // gph, u % gph
        tile = pl.multiple_of((it % nt) * T, T)
        cols = pl.ds(q_col(it), QB)
        qt = qt_ref[pl.ds(pl.multiple_of((it % nt) * (T // 2), T // 2), T // 2), cols]
        grp = lax.broadcasted_iota(jnp.int32, qt.shape, 0) // (dh // 2)
        w = _unpack(jnp.where(grp == g, qt, jnp.zeros_like(qt)))
        s = _dot(_unpack(k_ref[:, pl.ds(tile, T)]), w)
        s = swap8(s)
        p = jnp.exp2(s - jnp.max(s, axis=0, keepdims=True))
        lt = jnp.sum(p, axis=0, keepdims=True)
        o = _dot(_unpack(vt_ref[head_rows_packed(it, g), :]), p.astype(BF16))
        ot_ref[pl.ds(head_row(it, g), dh), cols] = o / lt
        return carry

    def layer(li, carry):
        def a_body(i, c):
            @pl.when(li == 0)
            def _():
                @pl.when(i + 1 < nrb)
                def _():
                    x_copy(i + 1).wait()

            qkv_block(li, i)
            return c

        lax.fori_loop(jnp.where(li == 0, 1, 0), nrb, a_body, 0)

        @pl.when(li == 0)
        def _():
            for j in range(4):
                w_copy(j).wait()

        for d, q in enumerate(q_bcast(0, 0)):
            qb_ref[d] = q
        bad_ref[...] = jnp.zeros_like(bad_ref)
        lax.fori_loop(0, nit, att_body, 0)

        def attempt(c):
            k, _ = c

            @pl.when(k == 1)
            def _():
                lax.fori_loop(0, nit * gph, att_safe_body, 0)

            unsafe = att_tail(k == 0) > 0.5
            wo_phase(li)
            return k + 1, unsafe

        lax.while_loop(lambda c: (c[0] == 0) | ((c[0] == 1) & c[1]), attempt, (0, False))

        def b_body(i, c):
            ffn_block(li, i)
            return c

        lax.fori_loop(0, nrb, b_body, 0)
        return carry

    lax.fori_loop(0, N_LAYERS, layer, 0)
    for i in range(nrb):
        for r in range(2):
            for q in range(2):
                out_copy(i, r, q).wait()


@jax.jit
def pallas_interleave_layers__softmax_full_mha__glu_gated_bilinear__prompt_kernel(
    A_x: jax.Array,
    A_wqkv: jax.Array,
    A_wo: jax.Array,
    B_x: jax.Array,
    B_w_gate: jax.Array,
    B_w_up: jax.Array,
    B_w_down: jax.Array,
):
    del B_x
    B, S, D = A_x.shape
    assert B == 1
    F = B_w_gate.shape[1]
    x2 = A_x.reshape(S, D)
    dh = D // N_HEADS
    fq = (F // T) // 4

    scratch = [
        pltpu.VMEM((S, D), A_x.dtype),
        pltpu.VMEM(A_wqkv.shape, A_wqkv.dtype),
        pltpu.VMEM(A_wo.shape, A_wo.dtype),
        pltpu.VMEM((2,) + B_w_gate.shape, B_w_gate.dtype),
        pltpu.VMEM(B_w_down.shape, B_w_down.dtype),
        pltpu.VMEM((3, 7, D // 4, D // 2), U32),
        pltpu.VMEM((7, D // 4, D // 2), U32),
        pltpu.VMEM((2, 49, T // 2, fq * T), U32),
        pltpu.VMEM((2, 14, T, T), U32),
        pltpu.VMEM((49, fq * T // 2, T), U32),
        pltpu.VMEM((7, T // 2, D // 2), U32),
        pltpu.VMEM((S, D), F32),
        pltpu.VMEM((S, D), F32),
        pltpu.VMEM((S // 4, 7 * D // 2), U32),
        pltpu.VMEM((S // 8, 49 * T), U32),
        pltpu.VMEM((S // 2, D), U32),
        pltpu.VMEM((S // T * 8, D), jnp.int32),
        pltpu.VMEM((D // 2, S), U32),
        pltpu.VMEM((D // 2, S), U32),
        pltpu.VMEM((D, S), F32),
        pltpu.VMEM((2, T, QB), F32),
        pltpu.VMEM((8, QB), F32),
        pltpu.VMEM((8, QB), F32),
        pltpu.VMEM((dh, QB), F32),
        pltpu.VMEM((dh, 8, QB), F32),
        pltpu.VMEM((T, 8, T), jnp.int32),
        pltpu.SMEM((2,), jnp.int32),
        pltpu.SemaphoreType.DMA((S // RB + 7,)),
    ]
    any_spec = pl.BlockSpec(memory_space=pl.ANY)
    out = pl.pallas_call(
        functools.partial(_kernel, S=S, D=D, F=F),
        out_shape=jax.ShapeDtypeStruct((S, D), A_x.dtype),
        in_specs=[any_spec] * 6,
        out_specs=any_spec,
        scratch_shapes=scratch,
        compiler_params=pltpu.CompilerParams(vmem_limit_bytes=100 * 1024 * 1024),
    )(x2, A_wqkv, A_wo, B_w_gate, B_w_up, B_w_down)
    return out.reshape(B, S, D)
```
